```python
import os as _os
_os.environ.setdefault('JAX_PLATFORMS', 'cpu')
import jax
import jax.numpy as jnp

def _softmax(x, axis=-1):
    return jax.nn.softmax(x, axis=axis)

def _gelu(x):
    return jax.nn.gelu(x, approximate=True)

def _silu(x):
    return jax.nn.silu(x)

def _sigmoid(x):
    return jax.nn.sigmoid(x)

def _layernorm(x, axis=-1, eps=1e-05):
    m = jnp.mean(x, axis=axis, keepdims=True)
    v = jnp.var(x, axis=axis, keepdims=True)
    return (x - m) / jnp.sqrt(v + eps)

def _scatter_add(tgt, idx, src, axis=0):
    return tgt.at[idx].add(src)

def _segment_sum(src, seg, n):
    return jax.ops.segment_sum(src, seg, n)

class _Rng:

    def __init__(self, key):
        self._k = key

    def _next(self):
        self._k, sub = jax.random.split(self._k)
        return sub

    def normal(self, shape):
        return jax.random.normal(self._next(), shape, dtype=jnp.bfloat16)

    def randint(self, lo, hi, shape):
        return jax.random.randint(self._next(), shape, lo, hi, dtype=jnp.int32)

    def uniform(self, shape, lo=0.0, hi=1.0):
        return jax.random.uniform(self._next(), shape, jnp.bfloat16, lo, hi)

    def permutation(self, n):
        return jax.random.permutation(self._next(), n)
kernel_name = 'adaLN_cond__softmax_full_mha__mixer_gmlp__prompt'

def setup_inputs():
    _rng = _Rng(jax.random.key(int.from_bytes(__import__("os").urandom(4), "little")))
    _w = lambda a: (lambda t: t.astype(jnp.bfloat16) if jnp.issubdtype(t.dtype, jnp.floating) else t)(jnp.asarray(a))

    def _A_setup():
        B, S, D = (1, 2048, 512)
        return {'x': _w((lambda *s: _rng.normal(s) * 0.05)(B, S, D)), 'wqkv': _w((lambda *s: _rng.normal(s) * 0.05)(D, 3 * D)), 'wo': _w((lambda *s: _rng.normal(s) * 0.05)(D, D))}
    _A_in = _A_setup()

    def _B_setup():
        B, S, D, F = (1, 2048, 512, 1792)
        Fh = F // 2
        return {'x': _w((lambda *s: _rng.normal(s) * 0.05)(B, S, D)), 'w_in': _w((lambda *s: _rng.normal(s) * 0.4)(D, 2 * Fh)), 'w_sp': _w(0.01 * (lambda *s: _rng.normal(s) * 0.4)(S, S)), 'b_sp': _w(1.0 + 0.01 * (lambda *s: _rng.normal(s) * 0.05)(S)), 'w_out': _w((lambda *s: _rng.normal(s) * 0.05)(Fh, D))}
    _B_in = _B_setup()
    return {'A_x': _A_in['x'], 'A_wqkv': _A_in['wqkv'], 'A_wo': _A_in['wo'], 'B_x': _B_in['x'], 'B_w_in': _B_in['w_in'], 'B_w_sp': _B_in['w_sp'], 'B_b_sp': _B_in['b_sp'], 'B_w_out': _B_in['w_out'], 'c': _w((lambda *s: _rng.normal(s) * 0.05)(1, 512) * 8.0), 'w_mod': _w((lambda *s: _rng.normal(s) * 0.05)(512, 6 * 512) * 512 ** (-0.5) * 8.0)}

def reference(A_x, A_wqkv, A_wo, B_x, B_w_in, B_w_sp, B_b_sp, B_w_out, c, w_mod):

    def _A_ref(x, wqkv, wo):
        B, S, D = x.shape
        H = 32
        Dh = D // H
        qkv = (lambda x, *d: x.transpose(*d))((x @ wqkv).reshape(B, S, 3, H, Dh), 2, 0, 3, 1, 4)
        q, k, v = (qkv[0], qkv[1], qkv[2])
        scale = Dh ** (-0.5)
        scores = jnp.einsum('bhqd,bhkd->bhqk', q, k) * scale
        p = _softmax(scores, axis=-1)
        o = jnp.einsum('bhqk,bhkd->bhqd', p, v)
        return (lambda x, *d: x.transpose(*d))(o, 0, 2, 1, 3).reshape(B, S, D) @ wo

    def _B_ref(x, w_in, w_sp, b_sp, w_out):
        B, S, D = x.shape
        F = w_in.shape[-1]
        Fh = F // 2
        z = _gelu(jnp.einsum('bsd,df->bsf', x, w_in))
        z1 = z[..., :Fh].copy()
        z2 = _layernorm(z[..., Fh:], axis=-1)
        g = jnp.einsum('ts,bsf->btf', w_sp, z2) + b_sp[None, :, None]
        return jnp.einsum('bsf,fd->bsd', z1 * g, w_out)
    x = A_x
    mod = (_silu(c) @ w_mod).reshape(c.shape[0], 6, 1, -1)
    sa, ca, ga, sb, cb, gb = (mod[:, 0].copy(), mod[:, 1].copy(), mod[:, 2].copy(), mod[:, 3].copy(), mod[:, 4].copy(), mod[:, 5].copy())
    h = _layernorm(x, axis=-1) * (1 + ca) + sa
    x = x + ga * _A_ref(h, A_wqkv, A_wo)
    h = _layernorm(x, axis=-1) * (1 + cb) + sb
    x = x + gb * _B_ref(h, B_w_in, B_w_sp, B_b_sp, B_w_out)
    return x
```

```python
import functools
import jax
import jax.numpy as jnp
from jax import lax
import jax.experimental.pallas as pl
import jax.experimental.pallas.tpu as pltpu

S = 2048
D = 512
H = 32
DH = 16
FH = 896
EPS = 1e-5
LOG2E = 1.4426950408889634
BF = jnp.bfloat16
F32 = jnp.float32
U32 = jnp.uint32

TB = 512
TQ = 512
CK = 128


def _ln(x):
    m = jnp.mean(x, axis=-1, keepdims=True)
    xc = x - m
    v = jnp.mean(xc * xc, axis=-1, keepdims=True)
    return xc * lax.rsqrt(v + EPS)


def _gelu(x):
    return 0.5 * x * (1.0 + jnp.tanh(0.7978845608028654 * (x + 0.044715 * (x * x * x))))


def _pack(x):
    return pltpu.bitcast(x.astype(BF), U32)


def _unpack(x):
    return pltpu.bitcast(x, BF)


def _kernel(c_ref, bsp_ref, x_hbm, wqkv_hbm, wo_hbm, win_hbm, wsp_hbm, wout_hbm, wmod_hbm, out_hbm,
            x_v, wqkv_v, wo_v, win_v, wsp_v, wout_v, wmod_v,
            mod_v, wqvT_v, k_v, qT_v, vT_v, s_v, oT_v, x1_v, z1_v, z2_v, out_v, sems, osems):
    cps = [
        pltpu.make_async_copy(wmod_hbm, wmod_v, sems.at[0]),
        pltpu.make_async_copy(x_hbm, x_v, sems.at[1]),
        pltpu.make_async_copy(wqkv_hbm, wqkv_v, sems.at[2]),
        pltpu.make_async_copy(wo_hbm, wo_v, sems.at[3]),
        pltpu.make_async_copy(win_hbm, win_v, sems.at[4]),
        pltpu.make_async_copy(wsp_hbm, wsp_v, sems.at[5]),
        pltpu.make_async_copy(wout_hbm, wout_v, sems.at[6]),
    ]
    for cp in cps:
        cp.start()

    cps[0].wait()
    c = c_ref[...].astype(F32)
    sc = c * jax.nn.sigmoid(c)
    sc8 = jnp.broadcast_to(sc, (8, D)).astype(BF)
    mod_v[...] = jnp.dot(sc8, wmod_v[...], preferred_element_type=F32)

    def mod(i):
        return mod_v[0:1, i * D:(i + 1) * D]

    cps[2].wait()
    wqvT_v[0:D // 2, :] = _pack(wqkv_v[:, 0:D].astype(F32).T)
    wqvT_v[D // 2:D, :] = _pack(wqkv_v[:, 2 * D:3 * D].astype(F32).T)

    cps[1].wait()
    qscale = (DH ** -0.5) * LOG2E

    def p1(b, carry):
        r0 = pl.multiple_of(b * TB, TB)
        x = x_v[pl.ds(r0, TB), :].astype(F32)
        h = (_ln(x) * (1.0 + mod(1)) + mod(0)).astype(BF)
        k = jnp.dot(h, wqkv_v[:, D:2 * D], preferred_element_type=F32)
        kp = _pack(k)
        r0h = pl.multiple_of(b * (TB // 2), TB // 2)
        for g in range(4):
            k_v[g, pl.ds(r0h, TB // 2), :] = kp[:, g * 128:(g + 1) * 128]
        qv = lax.dot_general(_unpack(wqvT_v[...]), h, (((1,), (1,)), ((), ())), preferred_element_type=F32)
        qT_v[b] = _pack(qv[0:D] * qscale)
        vT_v[b] = _pack(qv[D:2 * D])
        return carry

    lax.fori_loop(0, S // TB, p1, 0)

    NQ = S // TQ
    NC = S // CK
    rowgrp = lax.broadcasted_iota(jnp.int32, (64, TQ), 0) // 8

    def qweights(i):
        qb = i // H
        h = i % H
        g = h // 8
        blk = qT_v[qb, pl.ds(pl.multiple_of(g * 64, 64), 64), :]
        return _unpack(jnp.where(rowgrp == (h % 8), blk, jnp.zeros_like(blk))), g

    def qk_chunk(c, qw, g, mn):
        kc = _unpack(k_v[g, c * CK // 2:(c + 1) * CK // 2, :])
        s = jnp.dot(kc, qw, preferred_element_type=F32)
        s_v[c * CK:(c + 1) * CK, :] = s
        return jnp.maximum(mn, jnp.max(s.reshape(CK // 8, 8, TQ), axis=0))

    def pv_chunk(c, h, m, l, acc):
        p = jnp.exp2(s_v[c * CK:(c + 1) * CK, :] - m)
        l = l + jnp.sum(p.reshape(CK // 8, 8, TQ), axis=0)
        kb, off = divmod(c * CK, TB)
        vc = _unpack(vT_v[kb, pl.ds(pl.multiple_of(h * 8, 8), 8), off:off + CK])
        acc = acc + jnp.dot(vc, p.astype(BF), preferred_element_type=F32)
        return l, acc

    def finish(i, l, acc):
        qb = i // H
        h = i % H
        o = acc / jnp.sum(l, axis=0, keepdims=True)
        oT_v[qb, pl.ds(pl.multiple_of(h * 16, 16), 16), :] = o

    neg = jnp.full((8, TQ), -jnp.inf, F32)
    qw0, g0 = qweights(0)
    mn = neg
    for c in range(NC):
        mn = qk_chunk(c, qw0, g0, mn)
    m0 = jnp.max(mn, axis=0, keepdims=True)

    def att(i, m):
        qw, g = qweights(i + 1)
        h = i % H
        l = jnp.zeros((8, TQ), F32)
        acc = jnp.zeros((16, TQ), F32)
        mn = neg
        for c in range(NC):
            l, acc = pv_chunk(c, h, m, l, acc)
            mn = qk_chunk(c, qw, g, mn)
        finish(i, l, acc)
        return jnp.max(mn, axis=0, keepdims=True)

    m_last = lax.fori_loop(0, NQ * H - 1, att, m0)
    l = jnp.zeros((8, TQ), F32)
    acc = jnp.zeros((16, TQ), F32)
    for c in range(NC):
        l, acc = pv_chunk(c, H - 1, m_last, l, acc)
    finish(NQ * H - 1, l, acc)

    cps[3].wait()
    cps[4].wait()

    def p3(b, carry):
        r0 = pl.multiple_of(b * TB, TB)
        r0h = pl.multiple_of(b * (TB // 2), TB // 2)
        o = oT_v[b].T.astype(BF)
        a = jnp.dot(o, wo_v[...], preferred_element_type=F32)
        x1 = x_v[pl.ds(r0, TB), :].astype(F32) + mod(2) * a
        x1_v[pl.ds(r0, TB), :] = x1
        h2 = (_ln(x1) * (1.0 + mod(4)) + mod(3)).astype(BF)
        z1_v[pl.ds(r0, TB), :] = _gelu(jnp.dot(h2, win_v[:, 0:FH], preferred_element_type=F32))
        z2 = _gelu(jnp.dot(h2, win_v[:, FH:2 * FH], preferred_element_type=F32))
        z2_v[pl.ds(r0h, TB // 2), :] = _pack(_ln(z2))
        return carry

    lax.fori_loop(0, S // TB, p3, 0)

    cps[5].wait()
    cps[6].wait()

    def ocopy(b):
        r0 = pl.multiple_of(b * TB, TB)
        return pltpu.make_async_copy(out_v.at[pl.ds(r0, TB), :], out_hbm.at[pl.ds(r0, TB), :], osems.at[b])

    def p4(b, carry):
        r0 = pl.multiple_of(b * TB, TB)
        g = jnp.dot(wsp_v[pl.ds(r0, TB), :], _unpack(z2_v[...]), preferred_element_type=F32)
        bcol = jnp.broadcast_to(bsp_ref[b].astype(F32), (128, TB)).T
        g = g + jnp.concatenate([bcol] * (FH // 128), axis=1)
        u = (z1_v[pl.ds(r0, TB), :] * g).astype(BF)
        y = jnp.dot(u, wout_v[...], preferred_element_type=F32)
        out_v[pl.ds(r0, TB), :] = (x1_v[pl.ds(r0, TB), :] + mod(5) * y).astype(BF)
        ocopy(b).start()
        return carry

    lax.fori_loop(0, S // TB, p4, 0)
    for b in range(S // TB):
        ocopy(b).wait()


@jax.jit
def pallas_adaLN_cond__softmax_full_mha__mixer_gmlp__prompt_kernel(A_x, A_wqkv, A_wo, B_x, B_w_in, B_w_sp, B_b_sp, B_w_out, c, w_mod):
    assert TB == TQ
    x = A_x.reshape(S, D)
    bsp = B_b_sp.reshape(S // TB, 1, TB)
    any_spec = pl.BlockSpec(memory_space=pl.ANY)
    vm = pl.BlockSpec(memory_space=pltpu.VMEM)
    out = pl.pallas_call(
        _kernel,
        out_shape=jax.ShapeDtypeStruct((S, D), BF),
        in_specs=[vm, vm] + [any_spec] * 7,
        out_specs=any_spec,
        scratch_shapes=[
            pltpu.VMEM((S, D), BF), pltpu.VMEM((D, 3 * D), BF), pltpu.VMEM((D, D), BF),
            pltpu.VMEM((D, 2 * FH), BF), pltpu.VMEM((S, S), BF), pltpu.VMEM((FH, D), BF),
            pltpu.VMEM((D, 6 * D), BF),
            pltpu.VMEM((8, 6 * D), F32),
            pltpu.VMEM((D, D), U32),
            pltpu.VMEM((4, S // 2, 128), U32),
            pltpu.VMEM((S // TB, D // 2, TB), U32),
            pltpu.VMEM((S // TB, D // 2, TB), U32),
            pltpu.VMEM((S, TQ), F32),
            pltpu.VMEM((S // TQ, D, TQ), F32),
            pltpu.VMEM((S, D), F32),
            pltpu.VMEM((S, FH), F32),
            pltpu.VMEM((S // 2, FH), U32),
            pltpu.VMEM((S, D), BF),
            pltpu.SemaphoreType.DMA((7,)),
            pltpu.SemaphoreType.DMA((S // TB,)),
        ],
        compiler_params=pltpu.CompilerParams(vmem_limit_bytes=100 * 1024 * 1024),
    )(c, bsp, x, A_wqkv, A_wo, B_w_in, B_w_sp, B_w_out, w_mod)
    return out.reshape(1, S, D)
```

```python
import contextlib
import jax
import jax.numpy as jnp
from jax import lax
import jax.experimental.pallas as pl
import jax.experimental.pallas.tpu as pltpu

S = 2048
D = 512
H = 32
DH = 16
FH = 896
EPS = 1e-5
LOG2E = 1.4426950408889634
BF = jnp.bfloat16
F32 = jnp.float32
U32 = jnp.uint32

TB = 256
NB = S // TB
TB4 = 512
TQ = 512
CK = 128
NQ = S // TQ
NC = S // CK
NP = H // 2
NI = 2 * NQ
FEN = 2 * NC * DH
S_LIMIT = 80.0
V_LIMIT = 2.0 ** 20
FORCE_FALLBACK = False
PROF = False


def _scope(name):
    return jax.named_scope(name) if PROF else contextlib.nullcontext()


def _ln(x):
    m = jnp.mean(x, axis=-1, keepdims=True)
    xc = x - m
    v = jnp.mean(xc * xc, axis=-1, keepdims=True)
    return xc * lax.rsqrt(v + EPS)


def _gelu(x):
    hx = 0.5 * x
    return hx + hx * jnp.tanh(x * (0.7978845608028654 + (0.7978845608028654 * 0.044715) * (x * x)))


def _pack(x):
    return pltpu.bitcast(x.astype(BF), U32)


def _unpack(x):
    return pltpu.bitcast(x, BF)


def _pk(a, b):
    return pltpu.pack_elementwise([a, b], packed_dtype=BF)


def _upk(x, i):
    return pltpu.unpack_elementwise(x, index=i, packed_dtype=BF, unpacked_dtype=F32)


def _mo(x, n):
    return x if isinstance(x, int) else pl.multiple_of(x, n)


def _kernel(c_ref, bsp_ref, x_hbm, wqkv_hbm, wo_hbm, win_hbm, wsp_hbm, wout_hbm, wmod_hbm, out_hbm,
            x_v, wqkv_v, wo_v, win_v, wsp_v, wout_v, wmod_v,
            mod_v, wqvT_v, h_v, k_v, qT_v, vT_v, p_v, l_v, kba_v, kbb_v, qb_v, oT_v, bcol_v,
            x1_v, z1_v, z2_v, out_v, zero_s, sems, xsems, osems):
    def rows(b, n):
        return pl.ds(_mo(b * n, n), n)

    def xcopy(b):
        return pltpu.make_async_copy(x_hbm.at[rows(b, TB), :], x_v.at[rows(b, TB), :], xsems.at[b])

    cp_mod_a = pltpu.make_async_copy(wmod_hbm.at[:, 0:2 * D], wmod_v.at[:, 0:2 * D], sems.at[0])
    cp_wk = pltpu.make_async_copy(wqkv_hbm.at[:, D:2 * D], wqkv_v.at[:, D:2 * D], sems.at[1])
    cp_wq = pltpu.make_async_copy(wqkv_hbm.at[:, 0:D], wqkv_v.at[:, 0:D], sems.at[2])
    cp_wv = pltpu.make_async_copy(wqkv_hbm.at[:, 2 * D:3 * D], wqkv_v.at[:, 2 * D:3 * D], sems.at[3])
    cp_mod_b = pltpu.make_async_copy(wmod_hbm.at[:, 2 * D:6 * D], wmod_v.at[:, 2 * D:6 * D], sems.at[4])
    cp_wo = pltpu.make_async_copy(wo_hbm, wo_v, sems.at[5])
    cp_win = pltpu.make_async_copy(win_hbm, win_v, sems.at[6])
    cp_wsp = pltpu.make_async_copy(wsp_hbm, wsp_v, sems.at[7])
    cp_wout = pltpu.make_async_copy(wout_hbm, wout_v, sems.at[8])

    cp_mod_a.start()
    xcopy(0).start()
    cp_wk.start()
    zero_s[0] = 0

    c = c_ref[...].astype(F32)
    sc = c * jax.nn.sigmoid(c)
    sc8 = jnp.broadcast_to(sc, (8, D)).astype(BF)
    with _scope("w_moda"):
        cp_mod_a.wait()
    cp_wq.start()
    cp_wv.start()
    xcopy(1).start()
    mod_v[:, 0:2 * D] = jnp.dot(sc8, wmod_v[:, 0:2 * D], preferred_element_type=F32)

    def mod(i):
        return mod_v[0:1, i * D:(i + 1) * D]

    qscale = (DH ** -0.5) * LOG2E

    def ln1(b):
        xw = pltpu.bitcast(x_v[rows(b, TB), :], U32)
        he = _ln(_upk(xw, 0)) * (1.0 + mod(1)) + mod(0)
        ho = _ln(_upk(xw, 1)) * (1.0 + mod(1)) + mod(0)
        hn = _pk(he, ho)
        parts = []
        for g in range(TB // 16):
            if g % 8 == 7:
                parts.append(hn[g * 8:(g + 1) * 8])
            else:
                parts.append(_pack(jnp.concatenate([he[g * 8:(g + 1) * 8], ho[g * 8:(g + 1) * 8]], axis=0)))
        return hn, _unpack(jnp.concatenate(parts, axis=0))

    def kproj(b, hk, k2):
        k = jnp.dot(hk, wqkv_v[:, D:2 * D], preferred_element_type=F32)
        kp = _pack(k)
        for p in range(NP):
            blk = kp[:, (p // 4) * 128:(p // 4 + 1) * 128]
            if p % 4:
                blk = pltpu.roll(blk, 128 - 32 * (p % 4), 1)
            k_v[p, rows(b, TB // 2), :] = blk
        return jnp.maximum(k2, jnp.max((k * k).reshape(TB // 8, 8, D), axis=0))

    def qvproj(b, hn, q2, vm):
        qv = lax.dot_general(_unpack(wqvT_v[...]), _unpack(hn), (((1,), (1,)), ((), ())),
                             preferred_element_type=F32)
        q = qv[0:D] * qscale
        v = qv[D:2 * D]
        qT_v[b] = _pack(q)
        vp = _pack(v)
        for j in range(TB // CK):
            vT_v[b * (TB // CK) + j] = vp[:, j * CK:(j + 1) * CK]
        q2 = jnp.maximum(q2, jnp.sum((q * q).reshape(H, DH, TB), axis=1))
        vm = jnp.maximum(vm, jnp.max(jnp.abs(v).reshape(D // 8, 8, TB), axis=0))
        return q2, vm

    with _scope("ln0"):
        xcopy(0).wait()
        hn0, hk0 = ln1(0)
        h_v[...] = hn0
    with _scope("w_wk"):
        cp_wk.wait()
    with _scope("k0"):
        k2 = kproj(0, hk0, jnp.zeros((8, D), F32))
    with _scope("w_wqv"):
        cp_wq.wait()
        cp_wv.wait()
    for b in range(2, NB):
        xcopy(b).start()
    cp_mod_b.start()
    wqvT_v[0:D // 2, :] = _pack(wqkv_v[:, 0:D].astype(F32).T)
    wqvT_v[D // 2:D, :] = _pack(wqkv_v[:, 2 * D:3 * D].astype(F32).T)

    def p1(b, carry):
        k2, q2, vm = carry
        xcopy(b + 1).wait()
        hn = h_v[...]
        hn2, hk2 = ln1(b + 1)
        q2, vm = qvproj(b, hn, q2, vm)
        h_v[...] = hn2
        return kproj(b + 1, hk2, k2), q2, vm

    with _scope("p1"):
        k2, q2, vm = lax.fori_loop(0, NB - 1, p1, (k2, jnp.zeros((H, TB), F32), jnp.zeros((8, TB), F32)))

    zrows = jnp.zeros((8, TQ), U32)

    def qrows(pair, e, u):
        r = pl.ds(_mo(pair * 16 + e * 8, 8), 8)
        return jnp.concatenate([qT_v[2 * u, r, :], qT_v[2 * u + 1, r, :]], axis=1)

    def gen_kb(ref, pair, e, cg, b, ds):
        kf = _upk(k_v[pair, cg * 64 + 56:cg * 64 + 64, :], b)
        for d in ds:
            ref[(2 * cg + b) * DH + d] = jnp.broadcast_to(kf[:, e * DH + d:e * DH + d + 1], (8, 128))

    def gen_qb(slot, lo, hi, d):
        src = lo if d % 2 == 0 else hi
        qb_v[slot, d] = jnp.broadcast_to(src[d // 2:d // 2 + 1, :], (8, TQ))

    with _scope("p1_tail"):
        cp_mod_b.wait()
        for cp in (cp_wo, cp_win, cp_wsp, cp_wout):
            cp.start()
        q2, vm = qvproj(NB - 1, h_v[...], q2, vm)
        mod_v[:, 2 * D:6 * D] = jnp.dot(sc8, wmod_v[:, 2 * D:6 * D], preferred_element_type=F32)
        for cg in range(NC):
            for b in range(2):
                gen_kb(kba_v, 0, 0, cg, b, range(DH))
        for slot in range(NI - 1):
            w = qrows(0, slot // NQ, slot % NQ)
            lo, hi = _upk(w, 0), _upk(w, 1)
            for d in range(DH):
                gen_qb(slot, lo, hi, d)
        bs = bsp_ref[...].astype(F32)
        for j in range(S // 128):
            bcol_v[j * 128:(j + 1) * 128, :] = jnp.broadcast_to(bs[j:j + 1, :], (128, 128)).T

        k2 = jnp.max(k2, axis=0, keepdims=True)
        k2 = jnp.concatenate([k2[:, j * 128:(j + 1) * 128] for j in range(4)] * 2, axis=0)
        for sh in (1, 2, 4, 8):
            k2 = k2 + pltpu.roll(k2, sh, 1)
        lane = lax.broadcasted_iota(jnp.int32, (8, 128), 1)
        k2max = jnp.max(jnp.where(lane % 16 == 15, k2, 0.0))
        bound2 = jnp.max(q2) * k2max * 1.05
        safe = jnp.logical_and(bound2 <= S_LIMIT * S_LIMIT, jnp.max(vm) <= V_LIMIT)
        if FORCE_FALLBACK:
            safe = jnp.logical_and(safe, bound2 < 0.0)

    def put_o(head, u, o):
        r = pl.ds(_mo(head * DH, DH), DH)
        oT_v[2 * u, r, :] = o[:, :TB]
        oT_v[2 * u + 1, r, :] = o[:, TB:]

    def group(pp, dump, pq, pn, zero):
        pend = []
        for it in range(NI):
            e, u = divmod(it, NQ)
            kb_ref, kg_ref = (kba_v, kbb_v) if e == 0 else (kbb_v, kba_v)
            if pq is not None:
                blk = qrows(pq, e, u)
                qw = _unpack(jnp.concatenate([zrows, blk] if e else [blk, zrows], axis=0))
                gpair, ge = (pq, 1) if e == 0 else (pn, 0)
                slot = (it - 1) % NI
                w = qrows(pq if it == 0 else pn, slot // NQ, slot % NQ)
                qlo, qhi = _upk(w, 0), _upk(w, 1)
            lold = l_v[it]
            l = lv = acc = None
            for c in range(NC):
                x = p_v[it, c * 64:(c + 1) * 64, :]
                if pq is not None:
                    kc = _unpack(k_v[pq, c * 64:c * 64 + 56, :])[:, :2 * DH]
                    s = jnp.dot(kc, qw, preferred_element_type=F32)
                vc = _unpack(vT_v[c, pl.ds(_mo(pp * 16 + e * 8, 8), 8), :])
                d_ = jnp.dot(vc, _unpack(x), preferred_element_type=F32)
                acc = d_ if acc is None else d_ + acc
                if pq is not None:
                    for g in range(7):
                        p = jnp.exp2(s[g * 16:(g + 1) * 16])
                        t = p[:8] + p[8:]
                        l = t if l is None else l + t
                        p_v[it, c * 64 + g * 8:c * 64 + (g + 1) * 8, :] = _pk(p[:8], p[8:])
                    kb_ref[FEN + zero] = s[0:8, 0:128]
                    a = [None, None]
                    for d in range(DH):
                        qb = qb_v[it, d]
                        for b in range(2):
                            kb = kb_ref[(2 * c + b) * DH + d]
                            t = jnp.concatenate([kb] * (TQ // 128), axis=1) * qb
                            a[b] = t if a[b] is None else a[b] + t
                    a0 = jnp.exp2(a[0])
                    a1 = jnp.exp2(a[1])
                    lv = (a0 + a1) if lv is None else lv + (a0 + a1)
                    p_v[it, c * 64 + 56:c * 64 + 64, :] = _pk(a0, a1)
                if pend and c == 1:
                    pend.pop()()
                if pq is not None:
                    cg, part = divmod(u * NC + c, 4)
                    b, dh = divmod(part, 2)
                    gen_kb(kg_ref, gpair, ge, cg, b, range(dh * 8, dh * 8 + 8))
                    gen_qb(slot, qlo, qhi, c)

            def fin(it=it, e=e, u=u, acc=acc, l=l, lv=lv, lold=lold):
                put_o(pp * 2 + e, u if dump is None else jnp.where(dump, NQ, u),
                      acc / jnp.sum(lold, axis=0, keepdims=True))
                if pq is not None:
                    l_v[it] = l + lv

            if it < NI - 1:
                pend.append(fin)
            else:
                fin()

    @pl.when(safe)
    def _fast():
        zero = zero_s[0]

        def att(i, carry):
            group(jnp.maximum(i - 1, 0), i == 0, i, jnp.minimum(i + 1, NP - 1), zero)
            return carry

        with _scope("att_loop"):
            lax.fori_loop(0, NP, att, 0)
        with _scope("att_epi"):
            group(NP - 1, None, None, None, zero)

    @pl.when(jnp.logical_not(safe))
    def _exact_max():
        rgrp = lax.broadcasted_iota(jnp.int32, (16, TQ), 0) // 8

        def body(j, carry):
            h = j // NQ
            u = j % NQ
            pair = h // 2
            r = pl.ds(pl.multiple_of(pair * 16, 16), 16)
            blk = jnp.concatenate([qT_v[2 * u, r, :], qT_v[2 * u + 1, r, :]], axis=1)
            qw = _unpack(jnp.where(rgrp == h % 2, blk, jnp.zeros_like(blk)))

            def qk(c, mn):
                kc = _unpack(k_v[pair, rows(c, 64), :])[:, :2 * DH]
                s = jnp.dot(kc, qw, preferred_element_type=F32)
                p_v[c // 8, rows(c % 8, CK), :] = pltpu.bitcast(s, U32)
                return jnp.maximum(mn, jnp.max(s.reshape(CK // 8, 8, TQ), axis=0))

            mn = lax.fori_loop(0, NC, qk, jnp.full((8, TQ), -jnp.inf, F32))
            m = jnp.max(mn, axis=0, keepdims=True)

            def pv(c, carry):
                l, acc = carry
                x = pltpu.bitcast(p_v[c // 8, rows(c % 8, CK), :], F32)
                parts = []
                for g in range(8):
                    p = jnp.exp2(x[g * 16:(g + 1) * 16] - m)
                    l = l + (p[:8] + p[8:])
                    parts.append(_pk(p[:8], p[8:]) if g < 7 else _pack(p))
                pb = _unpack(jnp.concatenate(parts, axis=0))
                vc = _unpack(vT_v[c, rows(h, 8), :])
                return l, acc + jnp.dot(vc, pb, preferred_element_type=F32)

            l, acc = lax.fori_loop(0, NC, pv, (jnp.zeros((8, TQ), F32), jnp.zeros((DH, TQ), F32)))
            put_o(h, u, acc / jnp.sum(l, axis=0, keepdims=True))
            return carry

        lax.fori_loop(0, H * NQ, body, 0)

    cp_wo.wait()
    cp_win.wait()

    def p3a(b):
        o = oT_v[b].T.astype(BF)
        a = jnp.dot(o, wo_v[...], preferred_element_type=F32)
        x1 = x_v[rows(b, TB), :].astype(F32) + mod(2) * a
        x1_v[rows(b, TB), :] = x1
        return _pack(_ln(x1) * (1.0 + mod(4)) + mod(3))

    def p3b(b, h2):
        h2 = _unpack(h2)
        z2 = _gelu(jnp.dot(h2, win_v[:, FH:2 * FH], preferred_element_type=F32))
        z2_v[rows(b, TB // 2), :] = _pack(_ln(z2))
        z1_v[rows(b, TB), :] = _gelu(jnp.dot(h2, win_v[:, 0:FH], preferred_element_type=F32))

    def p3(b, carry):
        h2 = h_v[...]
        h2n = p3a(b + 1)
        p3b(b, h2)
        h_v[...] = h2n
        return carry

    with _scope("p3"):
        h_v[...] = p3a(0)
        lax.fori_loop(0, NB - 1, p3, 0)
        p3b(NB - 1, h_v[...])

    cp_wsp.wait()
    cp_wout.wait()

    def ocopy(b):
        return pltpu.make_async_copy(out_v.at[rows(b, TB4), :], out_hbm.at[rows(b, TB4), :], osems.at[b])

    def p4(b, carry):
        g = jnp.dot(wsp_v[rows(b, TB4), :], _unpack(z2_v[...]), preferred_element_type=F32)
        g = g + jnp.concatenate([bcol_v[rows(b, TB4), :]] * (FH // 128), axis=1)
        u = (z1_v[rows(b, TB4), :] * g).astype(BF)
        y = jnp.dot(u, wout_v[...], preferred_element_type=F32)
        out_v[rows(b, TB4), :] = (x1_v[rows(b, TB4), :] + mod(5) * y).astype(BF)
        ocopy(b).start()
        return carry

    with _scope("p4"):
        lax.fori_loop(0, S // TB4, p4, 0)
    with _scope("w_out"):
        for b in range(S // TB4):
            ocopy(b).wait()


@jax.jit
def pallas_adaLN_cond__softmax_full_mha__mixer_gmlp__prompt_kernel(A_x, A_wqkv, A_wo, B_x, B_w_in, B_w_sp, B_b_sp, B_w_out, c, w_mod):
    x = A_x.reshape(S, D)
    bsp = B_b_sp.reshape(S // 128, 128)
    any_spec = pl.BlockSpec(memory_space=pl.ANY)
    vm = pl.BlockSpec(memory_space=pltpu.VMEM)
    out = pl.pallas_call(
        _kernel,
        out_shape=jax.ShapeDtypeStruct((S, D), BF),
        in_specs=[vm, vm] + [any_spec] * 7,
        out_specs=any_spec,
        scratch_shapes=[
            pltpu.VMEM((S, D), BF), pltpu.VMEM((D, 3 * D), BF), pltpu.VMEM((D, D), BF),
            pltpu.VMEM((D, 2 * FH), BF), pltpu.VMEM((S, S), BF), pltpu.VMEM((FH, D), BF),
            pltpu.VMEM((D, 6 * D), BF),
            pltpu.VMEM((8, 6 * D), F32),
            pltpu.VMEM((D, D), U32),
            pltpu.VMEM((TB // 2, D), U32),
            pltpu.VMEM((NP, S // 2, 128), U32),
            pltpu.VMEM((NB, D // 2, TB), U32),
            pltpu.VMEM((NC, D // 2, CK), U32),
            pltpu.VMEM((NI, S // 2, TQ), U32),
            pltpu.VMEM((NI, 8, TQ), F32),
            pltpu.VMEM((FEN + 1, 8, 128), F32),
            pltpu.VMEM((FEN + 1, 8, 128), F32),
            pltpu.VMEM((NI, DH, 8, TQ), F32),
            pltpu.VMEM((NB + 2, D, TB), F32),
            pltpu.VMEM((S, 128), F32),
            pltpu.VMEM((S, D), F32),
            pltpu.VMEM((S, FH), F32),
            pltpu.VMEM((S // 2, FH), U32),
            pltpu.VMEM((S, D), BF),
            pltpu.SMEM((1,), jnp.int32),
            pltpu.SemaphoreType.DMA((9,)),
            pltpu.SemaphoreType.DMA((NB,)),
            pltpu.SemaphoreType.DMA((S // TB4,)),
        ],
        compiler_params=pltpu.CompilerParams(vmem_limit_bytes=110 * 1024 * 1024),
    )(c, bsp, x, A_wqkv, A_wo, B_w_in, B_w_sp, B_w_out, w_mod)
    return out.reshape(1, S, D)
```

```python
import contextlib
import jax
import jax.numpy as jnp
from jax import lax
import jax.experimental.pallas as pl
import jax.experimental.pallas.tpu as pltpu

S = 2048
D = 512
H = 32
DH = 16
FH = 896
EPS = 1e-5
LOG2E = 1.4426950408889634
BF = jnp.bfloat16
F32 = jnp.float32
U32 = jnp.uint32

TB = 256
NB = S // TB
TB4 = 512
TQ = 512
CK = 128
NQ = S // TQ
NC = S // CK
NP = H // 2
NI = 2 * NQ
FEN = 2 * NC * DH
S_LIMIT = 90.0
V_LIMIT = 2.0 ** 20
FORCE_FALLBACK = False
PROF = False


def _scope(name):
    return jax.named_scope(name) if PROF else contextlib.nullcontext()


def _ln(x):
    m = jnp.mean(x, axis=-1, keepdims=True)
    xc = x - m
    v = jnp.mean(xc * xc, axis=-1, keepdims=True)
    return xc * lax.rsqrt(v + EPS)


def _gelu(x):
    hx = 0.5 * x
    return hx + hx * jnp.tanh(x * (0.7978845608028654 + (0.7978845608028654 * 0.044715) * (x * x)))


def _pack(x):
    return pltpu.bitcast(x.astype(BF), U32)


def _unpack(x):
    return pltpu.bitcast(x, BF)


def _pk(a, b):
    return pltpu.pack_elementwise([a, b], packed_dtype=BF)


def _upk(x, i):
    return pltpu.unpack_elementwise(x, index=i, packed_dtype=BF, unpacked_dtype=F32)


def _mo(x, n):
    return x if isinstance(x, int) else pl.multiple_of(x, n)


def _kernel(c_ref, bsp_ref, x_hbm, wqkv_hbm, wo_hbm, win_hbm, wsp_hbm, wout_hbm, wmod_hbm, out_hbm,
            x_v, wqkv_v, wo_v, win_v, wsp_v, wout_v, wmod_v,
            mod_v, wqvT_v, h_v, k_v, qT_v, vT_v, p_v, l_v, kba_v, kbb_v, qb_v, oT_v, bcol_v,
            x1_v, z1_v, z2_v, out_v, zero_s, sems, xsems, osems):
    def rows(b, n):
        return pl.ds(_mo(b * n, n), n)

    def xcopy(b):
        return pltpu.make_async_copy(x_hbm.at[rows(b, TB), :], x_v.at[rows(b, TB), :], xsems.at[b])

    cp_mod_a = pltpu.make_async_copy(wmod_hbm.at[:, 0:2 * D], wmod_v.at[:, 0:2 * D], sems.at[0])
    cp_wk = pltpu.make_async_copy(wqkv_hbm.at[:, D:2 * D], wqkv_v.at[:, D:2 * D], sems.at[1])
    cp_wq = pltpu.make_async_copy(wqkv_hbm.at[:, 0:D], wqkv_v.at[:, 0:D], sems.at[2])
    cp_wv = pltpu.make_async_copy(wqkv_hbm.at[:, 2 * D:3 * D], wqkv_v.at[:, 2 * D:3 * D], sems.at[3])
    cp_mod_b = pltpu.make_async_copy(wmod_hbm.at[:, 2 * D:6 * D], wmod_v.at[:, 2 * D:6 * D], sems.at[4])
    cp_wo = pltpu.make_async_copy(wo_hbm, wo_v, sems.at[5])
    cp_win = pltpu.make_async_copy(win_hbm, win_v, sems.at[6])
    cp_wsp = pltpu.make_async_copy(wsp_hbm, wsp_v, sems.at[7])
    cp_wout = pltpu.make_async_copy(wout_hbm, wout_v, sems.at[8])

    cp_mod_a.start()
    xcopy(0).start()
    cp_wk.start()
    zero_s[0] = 0

    c = c_ref[...].astype(F32)
    sc = c * jax.nn.sigmoid(c)
    sc8 = jnp.broadcast_to(sc, (8, D)).astype(BF)
    with _scope("w_moda"):
        cp_mod_a.wait()
    cp_wq.start()
    cp_wv.start()
    xcopy(1).start()
    mod_v[:, 0:2 * D] = jnp.dot(sc8, wmod_v[:, 0:2 * D], preferred_element_type=F32)

    def mod(i):
        return mod_v[0:1, i * D:(i + 1) * D]

    qscale = (DH ** -0.5) * LOG2E

    def ln1(b):
        xw = pltpu.bitcast(x_v[rows(b, TB), :], U32)
        he = _ln(_upk(xw, 0)) * (1.0 + mod(1)) + mod(0)
        ho = _ln(_upk(xw, 1)) * (1.0 + mod(1)) + mod(0)
        hn = _pk(he, ho)
        parts = []
        for g in range(TB // 16):
            if g % 8 == 7:
                parts.append(hn[g * 8:(g + 1) * 8])
            else:
                parts.append(_pack(jnp.concatenate([he[g * 8:(g + 1) * 8], ho[g * 8:(g + 1) * 8]], axis=0)))
        return hn, _unpack(jnp.concatenate(parts, axis=0))

    def kproj(b, hk, k2):
        k = jnp.dot(hk, wqkv_v[:, D:2 * D], preferred_element_type=F32)
        kp = _pack(k)
        for p in range(NP):
            blk = kp[:, (p // 4) * 128:(p // 4 + 1) * 128]
            if p % 4:
                blk = pltpu.roll(blk, 128 - 32 * (p % 4), 1)
            k_v[p, rows(b, TB // 2), :] = blk
        return jnp.maximum(k2, jnp.max((k * k).reshape(TB // 8, 8, D), axis=0))

    def tproj(w, hn):
        return lax.dot_general(_unpack(w), _unpack(hn), (((1,), (1,)), ((), ())), preferred_element_type=F32)

    def qproj(b, hn, q2):
        q = tproj(wqvT_v[0:D // 2, :], hn) * qscale
        qT_v[b] = _pack(q)
        return jnp.maximum(q2, jnp.sum((q * q).reshape(H, DH, TB), axis=1))

    def vproj(b, hn, vm):
        v = tproj(wqvT_v[D // 2:D, :], hn)
        vp = _pack(v)
        for j in range(TB // CK):
            vT_v[b * (TB // CK) + j] = vp[:, j * CK:(j + 1) * CK]
        return jnp.maximum(vm, jnp.max(jnp.abs(v).reshape(D // 8, 8, TB), axis=0))

    with _scope("ln0"):
        xcopy(0).wait()
        hn0, hk0 = ln1(0)
        h_v[...] = hn0
    with _scope("w_wk"):
        cp_wk.wait()
    with _scope("k0"):
        k2 = kproj(0, hk0, jnp.zeros((8, D), F32))
    with _scope("w_wqv"):
        cp_wq.wait()
        cp_wv.wait()
    for b in range(2, NB):
        xcopy(b).start()
    cp_mod_b.start()
    wqvT_v[0:D // 2, :] = _pack(wqkv_v[:, 0:D].astype(F32).T)
    wqvT_v[D // 2:D, :] = _pack(wqkv_v[:, 2 * D:3 * D].astype(F32).T)

    def p1(b, carry):
        k2, q2, vm = carry
        xcopy(b + 1).wait()
        hn = h_v[...]
        hn2, hk2 = ln1(b + 1)
        q2 = qproj(b, hn, q2)
        k2 = kproj(b + 1, hk2, k2)
        vm = vproj(b, hn, vm)
        h_v[...] = hn2
        return k2, q2, vm

    with _scope("p1"):
        k2, q2, vm = lax.fori_loop(0, NB - 1, p1, (k2, jnp.zeros((H, TB), F32), jnp.zeros((8, TB), F32)))

    zrows = jnp.zeros((8, TQ), U32)

    def qrows(pair, e, u):
        r = pl.ds(_mo(pair * 16 + e * 8, 8), 8)
        return jnp.concatenate([qT_v[2 * u, r, :], qT_v[2 * u + 1, r, :]], axis=1)

    def gen_kb(ref, pair, e, cg, b, ds):
        kf = _upk(k_v[pair, cg * 64 + 56:cg * 64 + 64, :], b)
        for d in ds:
            ref[(2 * cg + b) * DH + d] = jnp.broadcast_to(kf[:, e * DH + d:e * DH + d + 1], (8, 128))

    def gen_qb(slot, lo, hi, d):
        src = lo if d % 2 == 0 else hi
        qb_v[slot, d] = jnp.broadcast_to(src[d // 2:d // 2 + 1, :], (8, TQ))

    with _scope("p1_tail"):
        cp_mod_b.wait()
        for cp in (cp_wo, cp_win, cp_wsp, cp_wout):
            cp.start()
        mod_v[:, 2 * D:6 * D] = jnp.dot(sc8, wmod_v[:, 2 * D:6 * D], preferred_element_type=F32)
        q2 = qproj(NB - 1, h_v[...], q2)
        vm = vproj(NB - 1, h_v[...], vm)
        for cg in range(NC):
            for b in range(2):
                gen_kb(kba_v, 0, 0, cg, b, range(DH))
        for slot in range(NI - 1):
            w = qrows(0, slot // NQ, slot % NQ)
            lo, hi = _upk(w, 0), _upk(w, 1)
            for d in range(DH):
                gen_qb(slot, lo, hi, d)
        bs = bsp_ref[...].astype(F32)
        for j in range(S // 128):
            bcol_v[j * 128:(j + 1) * 128, :] = jnp.broadcast_to(bs[j:j + 1, :], (128, 128)).T

        k2 = jnp.max(k2, axis=0, keepdims=True)
        k2 = jnp.concatenate([k2[:, j * 128:(j + 1) * 128] for j in range(4)] * 2, axis=0)
        for sh in (1, 2, 4, 8):
            k2 = k2 + pltpu.roll(k2, sh, 1)
        lane = lax.broadcasted_iota(jnp.int32, (8, 128), 1)
        k2max = jnp.max(jnp.where(lane % 16 == 15, k2, 0.0))
        bound2 = jnp.max(q2) * k2max * 1.05
        safe = jnp.logical_and(bound2 <= S_LIMIT * S_LIMIT, jnp.max(vm) <= V_LIMIT)
        if FORCE_FALLBACK:
            safe = jnp.logical_and(safe, bound2 < 0.0)

    def put_o(head, u, o):
        r = pl.ds(_mo(head * DH, DH), DH)
        oT_v[2 * u, r, :] = o[:, :TB]
        oT_v[2 * u + 1, r, :] = o[:, TB:]

    def group(pp, dump, pq, pn, zero):
        pend = []
        for it in range(NI):
            e, u = divmod(it, NQ)
            kb_ref, kg_ref = (kba_v, kbb_v) if e == 0 else (kbb_v, kba_v)
            if pq is not None:
                blk = qrows(pq, e, u)
                qw = _unpack(jnp.concatenate([zrows, blk] if e else [blk, zrows], axis=0))
                gpair, ge = (pq, 1) if e == 0 else (pn, 0)
                slot = (it - 1) % NI
                w = qrows(pq if it == 0 else pn, slot // NQ, slot % NQ)
                for i2 in range(2):
                    wf = _upk(w, i2)
                    for j in range(4):
                        kb_ref[FEN + 1 + 4 * i2 + j] = wf[:, j * 128:(j + 1) * 128]
                qdone = 0
            lold = l_v[it]
            l = lv = acc = None
            for c in range(NC):
                x = p_v[it, c * 64:(c + 1) * 64, :]
                if pq is not None:
                    kc = _unpack(k_v[pq, c * 64:c * 64 + 56, :])[:, :2 * DH]
                    s = jnp.dot(kc, qw, preferred_element_type=F32)
                vc = _unpack(vT_v[c, pl.ds(_mo(pp * 16 + e * 8, 8), 8), :])
                d_ = jnp.dot(vc, _unpack(x), preferred_element_type=F32)
                acc = d_ if acc is None else d_ + acc
                if pq is not None:
                    for g in range(7):
                        p = jnp.exp2(s[g * 16:(g + 1) * 16])
                        t = p[:8] + p[8:]
                        l = t if l is None else l + t
                        p_v[it, c * 64 + g * 8:c * 64 + (g + 1) * 8, :] = _pk(p[:8], p[8:])
                    a = [None, None]
                    for d in range(DH):
                        if d % 4 == 0:
                            kb_ref[FEN + zero] = s[(d // 2) * 16:(d // 2) * 16 + 8, 0:128]
                        qb = qb_v[it, d]
                        for b in range(2):
                            kb = kb_ref[(2 * c + b) * DH + d]
                            t = jnp.concatenate([kb] * (TQ // 128), axis=1) * qb
                            a[b] = t if a[b] is None else a[b] + t
                    a0 = jnp.exp2(a[0])
                    a1 = jnp.exp2(a[1])
                    lv = (a0 + a1) if lv is None else lv + (a0 + a1)
                    p_v[it, c * 64 + 56:c * 64 + 64, :] = _pk(a0, a1)
                if pend and c == 1:
                    pend.pop()()
                if pq is not None:
                    cg, part = divmod(u * NC + c, 4)
                    b, dh = divmod(part, 2)
                    gen_kb(kg_ref, gpair, ge, cg, b, range(dh * 8, dh * 8 + 8))
                    want = 0 if c < 2 else -(-DH * (c - 1) // (NC - 2))
                    for d in range(qdone, want):
                        src = jnp.concatenate([kb_ref[FEN + 1 + 4 * (d % 2) + j] for j in range(4)], axis=1)
                        gen_qb(slot, src, src, d)
                    qdone = want

            def fin(it=it, e=e, u=u, acc=acc, l=l, lv=lv, lold=lold):
                ls = jnp.sum(lold, axis=0, keepdims=True)
                r0 = pl.reciprocal(ls, approx=True)
                put_o(pp * 2 + e, u if dump is None else jnp.where(dump, NQ, u), acc * (r0 * (2.0 - ls * r0)))
                if pq is not None:
                    l_v[it] = l + lv

            if it < NI - 1:
                pend.append(fin)
            else:
                fin()

    @pl.when(safe)
    def _fast():
        zero = zero_s[0]

        def att(i, carry):
            group(jnp.maximum(i - 1, 0), i == 0, i, jnp.minimum(i + 1, NP - 1), zero)
            return carry

        with _scope("att_loop"):
            lax.fori_loop(0, NP, att, 0)
        with _scope("att_epi"):
            group(NP - 1, None, None, None, zero)

    @pl.when(jnp.logical_not(safe))
    def _exact_max():
        rgrp = lax.broadcasted_iota(jnp.int32, (16, TQ), 0) // 8

        def body(j, carry):
            h = j // NQ
            u = j % NQ
            pair = h // 2
            r = pl.ds(pl.multiple_of(pair * 16, 16), 16)
            blk = jnp.concatenate([qT_v[2 * u, r, :], qT_v[2 * u + 1, r, :]], axis=1)
            qw = _unpack(jnp.where(rgrp == h % 2, blk, jnp.zeros_like(blk)))

            def qk(c, mn):
                kc = _unpack(k_v[pair, rows(c, 64), :])[:, :2 * DH]
                s = jnp.dot(kc, qw, preferred_element_type=F32)
                p_v[c // 8, rows(c % 8, CK), :] = pltpu.bitcast(s, U32)
                return jnp.maximum(mn, jnp.max(s.reshape(CK // 8, 8, TQ), axis=0))

            mn = lax.fori_loop(0, NC, qk, jnp.full((8, TQ), -jnp.inf, F32))
            m = jnp.max(mn, axis=0, keepdims=True)

            def pv(c, carry):
                l, acc = carry
                x = pltpu.bitcast(p_v[c // 8, rows(c % 8, CK), :], F32)
                parts = []
                for g in range(8):
                    p = jnp.exp2(x[g * 16:(g + 1) * 16] - m)
                    l = l + (p[:8] + p[8:])
                    parts.append(_pk(p[:8], p[8:]) if g < 7 else _pack(p))
                pb = _unpack(jnp.concatenate(parts, axis=0))
                vc = _unpack(vT_v[c, rows(h, 8), :])
                return l, acc + jnp.dot(vc, pb, preferred_element_type=F32)

            l, acc = lax.fori_loop(0, NC, pv, (jnp.zeros((8, TQ), F32), jnp.zeros((DH, TQ), F32)))
            put_o(h, u, acc / jnp.sum(l, axis=0, keepdims=True))
            return carry

        lax.fori_loop(0, H * NQ, body, 0)

    cp_wo.wait()
    cp_win.wait()

    def p3a(b):
        o = oT_v[b].T.astype(BF)
        a = jnp.dot(o, wo_v[...], preferred_element_type=F32)
        x1 = x_v[rows(b, TB), :].astype(F32) + mod(2) * a
        x1_v[rows(b, TB), :] = x1
        return _pack(_ln(x1) * (1.0 + mod(4)) + mod(3))

    def p3z2(b, h2):
        z2 = _gelu(jnp.dot(_unpack(h2), win_v[:, FH:2 * FH], preferred_element_type=F32))
        z2_v[rows(b, TB // 2), :] = _pack(_ln(z2))

    def p3z1(b, h2):
        z1_v[rows(b, TB), :] = _gelu(jnp.dot(_unpack(h2), win_v[:, 0:FH], preferred_element_type=F32))

    def p3(b, carry):
        h2 = h_v[...]
        p3z2(b, h2)
        h2n = p3a(b + 1)
        p3z1(b, h2)
        h_v[...] = h2n
        return carry

    with _scope("p3"):
        h_v[...] = p3a(0)
        lax.fori_loop(0, NB - 1, p3, 0)
        p3z2(NB - 1, h_v[...])
        p3z1(NB - 1, h_v[...])

    cp_wsp.wait()
    cp_wout.wait()

    def ocopy(b):
        return pltpu.make_async_copy(out_v.at[rows(b, TB4), :], out_hbm.at[rows(b, TB4), :], osems.at[b])

    def p4(b, carry):
        g = jnp.dot(wsp_v[rows(b, TB4), :], _unpack(z2_v[...]), preferred_element_type=F32)
        g = g + jnp.concatenate([bcol_v[rows(b, TB4), :]] * (FH // 128), axis=1)
        u = (z1_v[rows(b, TB4), :] * g).astype(BF)
        y = jnp.dot(u, wout_v[...], preferred_element_type=F32)
        out_v[rows(b, TB4), :] = (x1_v[rows(b, TB4), :] + mod(5) * y).astype(BF)
        ocopy(b).start()
        return carry

    with _scope("p4"):
        lax.fori_loop(0, S // TB4, p4, 0)
    with _scope("w_out"):
        for b in range(S // TB4):
            ocopy(b).wait()


@jax.jit
def pallas_adaLN_cond__softmax_full_mha__mixer_gmlp__prompt_kernel(A_x, A_wqkv, A_wo, B_x, B_w_in, B_w_sp, B_b_sp, B_w_out, c, w_mod):
    x = A_x.reshape(S, D)
    bsp = B_b_sp.reshape(S // 128, 128)
    any_spec = pl.BlockSpec(memory_space=pl.ANY)
    vm = pl.BlockSpec(memory_space=pltpu.VMEM)
    out = pl.pallas_call(
        _kernel,
        out_shape=jax.ShapeDtypeStruct((S, D), BF),
        in_specs=[vm, vm] + [any_spec] * 7,
        out_specs=any_spec,
        scratch_shapes=[
            pltpu.VMEM((S, D), BF), pltpu.VMEM((D, 3 * D), BF), pltpu.VMEM((D, D), BF),
            pltpu.VMEM((D, 2 * FH), BF), pltpu.VMEM((S, S), BF), pltpu.VMEM((FH, D), BF),
            pltpu.VMEM((D, 6 * D), BF),
            pltpu.VMEM((8, 6 * D), F32),
            pltpu.VMEM((D, D), U32),
            pltpu.VMEM((TB // 2, D), U32),
            pltpu.VMEM((NP, S // 2, 128), U32),
            pltpu.VMEM((NB, D // 2, TB), U32),
            pltpu.VMEM((NC, D // 2, CK), U32),
            pltpu.VMEM((NI, S // 2, TQ), U32),
            pltpu.VMEM((NI, 8, TQ), F32),
            pltpu.VMEM((FEN + 9, 8, 128), F32),
            pltpu.VMEM((FEN + 9, 8, 128), F32),
            pltpu.VMEM((NI, DH, 8, TQ), F32),
            pltpu.VMEM((NB + 2, D, TB), F32),
            pltpu.VMEM((S, 128), F32),
            pltpu.VMEM((S, D), F32),
            pltpu.VMEM((S, FH), F32),
            pltpu.VMEM((S // 2, FH), U32),
            pltpu.VMEM((S, D), BF),
            pltpu.SMEM((1,), jnp.int32),
            pltpu.SemaphoreType.DMA((9,)),
            pltpu.SemaphoreType.DMA((NB,)),
            pltpu.SemaphoreType.DMA((S // TB4,)),
        ],
        compiler_params=pltpu.CompilerParams(vmem_limit_bytes=110 * 1024 * 1024),
    )(c, bsp, x, A_wqkv, A_wo, B_w_in, B_w_sp, B_w_out, w_mod)
    return out.reshape(1, S, D)
```

```python
import contextlib
import jax
import jax.numpy as jnp
from jax import lax
import jax.experimental.pallas as pl
import jax.experimental.pallas.tpu as pltpu

S = 2048
D = 512
H = 32
DH = 16
FH = 896
EPS = 1e-5
LOG2E = 1.4426950408889634
BF = jnp.bfloat16
F32 = jnp.float32
U32 = jnp.uint32

TB = 256
NB = S // TB
TB4 = 512
TQ = 512
CK = 128
NQ = S // TQ
NC = S // CK
NP = H // 2
NI = 2 * NQ
FEN = 2 * NC * DH
S_LIMIT = 90.0
V_LIMIT = 2.0 ** 20
KP = 384
WO_STEPS = (0, 2, 4, 6, 8, 10, 12, 13, 14)
WO_STEPS0 = (4, 6, 8, 10, 11, 12, 13, 14, 15)
WO_ROWS = (0, 96, 192, 256)
FORCE_FALLBACK = False
PROF = False


def _scope(name):
    return jax.named_scope(name) if PROF else contextlib.nullcontext()


def _ln(x):
    m = jnp.mean(x, axis=-1, keepdims=True)
    xc = x - m
    v = jnp.mean(xc * xc, axis=-1, keepdims=True)
    return xc * lax.rsqrt(v + EPS)


def _gelu(x):
    hx = 0.5 * x
    return hx + hx * jnp.tanh(x * (0.7978845608028654 + (0.7978845608028654 * 0.044715) * (x * x)))


def _pack(x):
    return pltpu.bitcast(x.astype(BF), U32)


def _unpack(x):
    return pltpu.bitcast(x, BF)


def _pk(a, b):
    return pltpu.pack_elementwise([a, b], packed_dtype=BF)


def _upk(x, i):
    return pltpu.unpack_elementwise(x, index=i, packed_dtype=BF, unpacked_dtype=F32)


def _mo(x, n):
    return x if isinstance(x, int) else pl.multiple_of(x, n)


def _kernel(c_hbm, bsp_hbm, x_hbm, wqkv_hbm, wo_hbm, win_hbm, wsp_hbm, wout_hbm, wmod_hbm, out_hbm,
            x_v, wqkv_v, wo_v, win_v, wsp_v, wout_v, wmod_v,
            mod_v, wqvT_v, h_v, k_v, qT_v, vT_v, p_v, l_v, kba_v, kbb_v, qb_v, oT_v, bcol_v,
            x1_v, z1_v, zg_v, z2_v, out_v, c_ref, bsp_ref, zero_s, sems, xsems, osems):
    def rows(b, n):
        return pl.ds(_mo(b * n, n), n)

    def xcopy(b):
        return pltpu.make_async_copy(x_hbm.at[rows(b, TB), :], x_v.at[rows(b, TB), :], xsems.at[b])

    cp_mod_a = pltpu.make_async_copy(wmod_hbm.at[:, 0:2 * D], wmod_v.at[:, 0:2 * D], sems.at[0])
    cp_wk = pltpu.make_async_copy(wqkv_hbm.at[:, D:2 * D], wqkv_v.at[:, D:2 * D], sems.at[1])
    cp_wq = pltpu.make_async_copy(wqkv_hbm.at[:, 0:D], wqkv_v.at[:, 0:D], sems.at[2])
    cp_wv = pltpu.make_async_copy(wqkv_hbm.at[:, 2 * D:3 * D], wqkv_v.at[:, 2 * D:3 * D], sems.at[3])
    cp_mod_b = pltpu.make_async_copy(wmod_hbm.at[:, 2 * D:6 * D], wmod_v.at[:, 2 * D:6 * D], sems.at[4])
    cp_wo = pltpu.make_async_copy(wo_hbm, wo_v, sems.at[5])
    cp_win = pltpu.make_async_copy(win_hbm, win_v, sems.at[6])
    cp_wsp = pltpu.make_async_copy(wsp_hbm, wsp_v, sems.at[7])
    cp_wout = pltpu.make_async_copy(wout_hbm, wout_v, sems.at[8])

    cp_c = pltpu.make_async_copy(c_hbm, c_ref, sems.at[9])
    cp_bsp = pltpu.make_async_copy(bsp_hbm, bsp_ref, sems.at[10])

    cp_mod_a.start()
    cp_c.start()
    xcopy(0).start()
    cp_wq.start()
    zero_s[0] = 0

    cp_c.wait()
    c = c_ref[...].astype(F32)
    sc = c * jax.nn.sigmoid(c)
    sc8 = jnp.broadcast_to(sc, (8, D)).astype(BF)
    with _scope("w_moda"):
        cp_mod_a.wait()
    cp_wk.start()
    cp_wv.start()
    xcopy(1).start()
    mod_v[:, 0:2 * D] = jnp.dot(sc8, wmod_v[:, 0:2 * D], preferred_element_type=F32)

    def mod(i):
        return mod_v[0:1, i * D:(i + 1) * D]

    qscale = (DH ** -0.5) * LOG2E

    def ln1(b):
        xw = pltpu.bitcast(x_v[rows(b, TB), :], U32)
        he = _ln(_upk(xw, 0)) * (1.0 + mod(1)) + mod(0)
        ho = _ln(_upk(xw, 1)) * (1.0 + mod(1)) + mod(0)
        hn = _pk(he, ho)
        parts = []
        for g in range(TB // 16):
            if g % 8 == 7:
                parts.append(hn[g * 8:(g + 1) * 8])
            else:
                parts.append(_pack(jnp.concatenate([he[g * 8:(g + 1) * 8], ho[g * 8:(g + 1) * 8]], axis=0)))
        return hn, _unpack(jnp.concatenate(parts, axis=0))

    def kproj(b, hk, k2):
        k = jnp.dot(hk, wqkv_v[:, D:2 * D], preferred_element_type=F32)
        kp = _pack(k)
        for p in range(NP):
            blk = kp[:, (p // 4) * 128:(p // 4 + 1) * 128]
            if p % 4:
                blk = pltpu.roll(blk, 128 - 32 * (p % 4), 1)
            k_v[p, rows(b, TB // 2), :] = blk
        return jnp.maximum(k2, jnp.max((k * k).reshape(TB // 8, 8, D), axis=0))

    def tproj(w, hn):
        return lax.dot_general(_unpack(w), _unpack(hn), (((1,), (1,)), ((), ())), preferred_element_type=F32)

    def qproj(b, hn, q2):
        q = tproj(wqvT_v[0:D // 2, :], hn) * qscale
        qT_v[b] = _pack(q)
        return jnp.maximum(q2, jnp.sum((q * q).reshape(H, DH, TB), axis=1))

    def vproj(b, hn, vm):
        v = tproj(wqvT_v[D // 2:D, :], hn)
        vp = _pack(v)
        for j in range(TB // CK):
            vT_v[b * (TB // CK) + j] = vp[:, j * CK:(j + 1) * CK]
        return jnp.maximum(vm, jnp.max(jnp.abs(v).reshape(D // 8, 8, TB), axis=0))

    with _scope("w_x0"):
        xcopy(0).wait()
        cp_wq.wait()
    with _scope("q0"):
        hn0, hk0 = ln1(0)
        wqvT_v[0:D // 2, :] = _pack(wqkv_v[:, 0:D].astype(F32).T)
        q2 = qproj(0, hn0, jnp.zeros((H, TB), F32))
    with _scope("w_wkv"):
        cp_wk.wait()
        cp_wv.wait()
        xcopy(1).wait()
    for b in range(2, NB):
        xcopy(b).start()
    cp_mod_b.start()
    cp_bsp.start()
    cp_wo.start()
    with _scope("kv0"):
        k2 = kproj(0, hk0, jnp.zeros((8, D), F32))
        wqvT_v[D // 2:D, :] = _pack(wqkv_v[:, 2 * D:3 * D].astype(F32).T)
        hn1, hk1 = ln1(1)
        h_v[...] = hn1
        vm = vproj(0, hn0, jnp.zeros((8, TB), F32))
        k2 = kproj(1, hk1, k2)

    def p1(b, carry):
        k2, q2, vm = carry
        xcopy(b + 1).wait()
        hn = h_v[...]
        hn2, hk2 = ln1(b + 1)
        q2 = qproj(b, hn, q2)
        k2 = kproj(b + 1, hk2, k2)
        vm = vproj(b, hn, vm)
        h_v[...] = hn2
        return k2, q2, vm

    with _scope("p1"):
        k2, q2, vm = lax.fori_loop(1, NB - 1, p1, (k2, q2, vm))

    zrows = jnp.zeros((8, TQ), U32)

    def qrows(pair, e, u):
        r = pl.ds(_mo(pair * 16 + e * 8, 8), 8)
        return jnp.concatenate([qT_v[2 * u, r, :], qT_v[2 * u + 1, r, :]], axis=1)

    def gen_kb(ref, pair, e, cg, b, ds):
        kf = _upk(k_v[pair, cg * 64 + 56:cg * 64 + 64, :], b)
        for d in ds:
            ref[(2 * cg + b) * DH + d] = jnp.broadcast_to(kf[:, e * DH + d:e * DH + d + 1], (8, 128))

    def gen_qb(slot, lo, hi, d):
        src = lo if d % 2 == 0 else hi
        qb_v[slot, d] = jnp.broadcast_to(src[d // 2:d // 2 + 1, :], (8, TQ))

    with _scope("p1_tail"):
        cp_mod_b.wait()
        cp_bsp.wait()
        cp_wo.wait()
        for cp in (cp_win, cp_wsp, cp_wout):
            cp.start()
        mod_v[:, 2 * D:6 * D] = jnp.dot(sc8, wmod_v[:, 2 * D:6 * D], preferred_element_type=F32)
        q2 = qproj(NB - 1, h_v[...], q2)
        vm = vproj(NB - 1, h_v[...], vm)
        for cg in range(NC):
            for b in range(2):
                gen_kb(kba_v, 0, 0, cg, b, range(DH))
        for slot in range(NI - 1):
            w = qrows(0, slot // NQ, slot % NQ)
            lo, hi = _upk(w, 0), _upk(w, 1)
            for d in range(DH):
                gen_qb(slot, lo, hi, d)
        bs = bsp_ref[...].astype(F32)
        for j in range(S // 128):
            bcol_v[j * 128:(j + 1) * 128, :] = jnp.broadcast_to(bs[j:j + 1, :], (128, 128)).T

        k2 = jnp.max(k2, axis=0, keepdims=True)
        k2 = jnp.concatenate([k2[:, j * 128:(j + 1) * 128] for j in range(4)] * 2, axis=0)
        for sh in (1, 2, 4, 8):
            k2 = k2 + pltpu.roll(k2, sh, 1)
        lane = lax.broadcasted_iota(jnp.int32, (8, 128), 1)
        k2max = jnp.max(jnp.where(lane % 16 == 15, k2, 0.0))
        bound2 = jnp.max(q2) * k2max * 1.05
        safe = jnp.logical_and(bound2 <= S_LIMIT * S_LIMIT, jnp.max(vm) <= V_LIMIT)
        if FORCE_FALLBACK:
            safe = jnp.logical_and(safe, bound2 < 0.0)

    zero3 = zero_s[0]
    RG = 16

    def outs(z, j, n):
        t = j * 6 * (z.shape[1] // 128) * (TB // 8) // (10 * n)
        nt, r = divmod(t, TB // 8)
        return z[r * 8:(r + 1) * 8, nt * 128:(nt + 1) * 128]

    def p3wo(b):
        o = oT_v[b, KP:D, :].T.astype(BF)
        a = jnp.dot(o, wo_v[KP:D, :], preferred_element_type=F32)
        x1_v[rows(b, TB), :] = x1_v[rows(b, TB), :] + mod(2) * a

    def ln_x1(b, pace):
        for j in range(TB // RG):
            if pace is not None:
                x1_v[pl.ds(pl.multiple_of(S + zero3 * 8, 8), 8), 0:128] = outs(pace, j, TB // RG)
            x1 = x1_v[pl.ds(_mo(b * TB + j * RG, RG), RG), :]
            h_v[j * RG // 2:(j + 1) * RG // 2, :] = _pack(_ln(x1) * (1.0 + mod(4)) + mod(3))

    def put_o(head, u, o):
        r = pl.ds(_mo(head * DH, DH), DH)
        oT_v[2 * u, r, :] = o[:, :TB]
        oT_v[2 * u + 1, r, :] = o[:, TB:]

    def group(pp, dump, pq, pn, zero):
        pend = []
        for pos in range(NI):
            it = pos if pq is not None else (pos % 2) * NQ + pos // 2
            e, u = divmod(it, NQ)
            if pq is None and pos == 3:
                p3wo(0)
                ln_x1(0, None)
            kb_ref, kg_ref = (kba_v, kbb_v) if e == 0 else (kbb_v, kba_v)
            if pq is not None:
                blk = qrows(pq, e, u)
                qw = _unpack(jnp.concatenate([zrows, blk] if e else [blk, zrows], axis=0))
                gpair, ge = (pq, 1) if e == 0 else (pn, 0)
                slot = (it - 1) % NI
                w = qrows(pq if it == 0 else pn, slot // NQ, slot % NQ)
                for i2 in range(2):
                    wf = _upk(w, i2)
                    for j in range(4):
                        kb_ref[FEN + 1 + 4 * i2 + j] = wf[:, j * 128:(j + 1) * 128]
                qdone = 0
            lold = l_v[it]
            l = lv = acc = None
            if pq is None:
                ob = oT_v[pos, 0:KP, :].T.astype(BF)
                wacc = None
            for c in range(NC):
                wsteps = WO_STEPS if pos else WO_STEPS0
                if pq is None and c in wsteps:
                    rb, kt = divmod(wsteps.index(c), KP // 128)
                    r0, r1 = WO_ROWS[rb], WO_ROWS[rb + 1]
                    w_ = jnp.dot(ob[r0:r1, kt * 128:(kt + 1) * 128],
                                 wo_v[kt * 128:(kt + 1) * 128, :], preferred_element_type=F32)
                    wacc = w_ if kt == 0 else w_ + wacc
                    if kt == KP // 128 - 1:
                        r = slice(pos * TB + r0, pos * TB + r1)
                        x1_v[r, :] = x_v[r, :].astype(F32) + mod(2) * wacc
                x = p_v[it, c * 64:(c + 1) * 64, :]
                if pq is not None:
                    kc = _unpack(k_v[pq, c * 64:c * 64 + 56, :])[:, :2 * DH]
                    s = jnp.dot(kc, qw, preferred_element_type=F32)
                vc = _unpack(vT_v[c, pl.ds(_mo(pp * 16 + e * 8, 8), 8), :])
                d_ = jnp.dot(vc, _unpack(x), preferred_element_type=F32)
                acc = d_ if acc is None else d_ + acc
                if pq is not None:
                    for g in range(7):
                        p = jnp.exp2(s[g * 16:(g + 1) * 16])
                        t = p[:8] + p[8:]
                        l = t if l is None else l + t
                        p_v[it, c * 64 + g * 8:c * 64 + (g + 1) * 8, :] = _pk(p[:8], p[8:])
                    a = [None, None]
                    for d in range(DH):
                        if d % 4 == 0:
                            kb_ref[FEN + zero] = s[(d // 2) * 16:(d // 2) * 16 + 8, 0:128]
                        qb = qb_v[it, d]
                        for b in range(2):
                            kb = kb_ref[(2 * c + b) * DH + d]
                            t = jnp.concatenate([kb] * (TQ // 128), axis=1) * qb
                            a[b] = t if a[b] is None else a[b] + t
                    a0 = jnp.exp2(a[0])
                    a1 = jnp.exp2(a[1])
                    lv = (a0 + a1) if lv is None else lv + (a0 + a1)
                    p_v[it, c * 64 + 56:c * 64 + 64, :] = _pk(a0, a1)
                if pend and c == 1:
                    pend.pop()()
                if pq is not None:
                    cg, part = divmod(u * NC + c, 4)
                    b, dh = divmod(part, 2)
                    gen_kb(kg_ref, gpair, ge, cg, b, range(dh * 8, dh * 8 + 8))
                    want = 0 if c < 2 else -(-DH * (c - 1) // (NC - 2))
                    for d in range(qdone, want):
                        src = jnp.concatenate([kb_ref[FEN + 1 + 4 * (d % 2) + j] for j in range(4)], axis=1)
                        gen_qb(slot, src, src, d)
                    qdone = want

            def fin(it=it, e=e, u=u, acc=acc, l=l, lv=lv, lold=lold):
                ls = jnp.sum(lold, axis=0, keepdims=True)
                r0 = pl.reciprocal(ls, approx=True)
                put_o(pp * 2 + e, u if dump is None else jnp.where(dump, NQ, u), acc * (r0 * (2.0 - ls * r0)))
                if pq is not None:
                    l_v[it] = l + lv

            if pos < NI - 1:
                pend.append(fin)
            else:
                fin()

    @pl.when(safe)
    def _fast():
        zero = zero_s[0]

        def att(i, carry):
            group(jnp.maximum(i - 1, 0), i == 0, i, jnp.minimum(i + 1, NP - 1), zero)
            return carry

        with _scope("att_loop"):
            lax.fori_loop(0, NP, att, 0)
        with _scope("att_epi"):
            group(NP - 1, None, None, None, zero)

    @pl.when(jnp.logical_not(safe))
    def _exact_max():
        rgrp = lax.broadcasted_iota(jnp.int32, (16, TQ), 0) // 8

        def body(j, carry):
            h = j // NQ
            u = j % NQ
            pair = h // 2
            r = pl.ds(pl.multiple_of(pair * 16, 16), 16)
            blk = jnp.concatenate([qT_v[2 * u, r, :], qT_v[2 * u + 1, r, :]], axis=1)
            qw = _unpack(jnp.where(rgrp == h % 2, blk, jnp.zeros_like(blk)))

            def qk(c, mn):
                kc = _unpack(k_v[pair, rows(c, 64), :])[:, :2 * DH]
                s = jnp.dot(kc, qw, preferred_element_type=F32)
                p_v[c // 8, rows(c % 8, CK), :] = pltpu.bitcast(s, U32)
                return jnp.maximum(mn, jnp.max(s.reshape(CK // 8, 8, TQ), axis=0))

            mn = lax.fori_loop(0, NC, qk, jnp.full((8, TQ), -jnp.inf, F32))
            m = jnp.max(mn, axis=0, keepdims=True)

            def pv(c, carry):
                l, acc = carry
                x = pltpu.bitcast(p_v[c // 8, rows(c % 8, CK), :], F32)
                parts = []
                for g in range(8):
                    p = jnp.exp2(x[g * 16:(g + 1) * 16] - m)
                    l = l + (p[:8] + p[8:])
                    parts.append(_pk(p[:8], p[8:]) if g < 7 else _pack(p))
                pb = _unpack(jnp.concatenate(parts, axis=0))
                vc = _unpack(vT_v[c, rows(h, 8), :])
                return l, acc + jnp.dot(vc, pb, preferred_element_type=F32)

            l, acc = lax.fori_loop(0, NC, pv, (jnp.zeros((8, TQ), F32), jnp.zeros((DH, TQ), F32)))
            put_o(h, u, acc / jnp.sum(l, axis=0, keepdims=True))
            return carry

        lax.fori_loop(0, H * NQ, body, 0)

        def wo_part(b, carry):
            a = jnp.dot(oT_v[b, 0:KP, :].T.astype(BF), wo_v[0:KP, :], preferred_element_type=F32)
            x1_v[rows(b, TB), :] = x_v[rows(b, TB), :].astype(F32) + mod(2) * a
            return carry

        lax.fori_loop(0, NB, wo_part, 0)
        p3wo(0)
        ln_x1(0, None)

    cp_win.wait()

    def ln_zg(b, pace):
        for j in range(TB // RG):
            if pace is not None:
                zg_v[pl.ds(pl.multiple_of(TB + zero3 * 8, 8), 8), 0:128] = outs(pace, j, TB // RG)
            z2_v[pl.ds(_mo(b * (TB // 2) + j * (RG // 2), RG // 2), RG // 2), :] = _pack(_ln(zg_v[j * RG:(j + 1) * RG, :]))

    def p3z(h2, lo):
        return _gelu(jnp.dot(_unpack(h2), win_v[:, lo:lo + FH], preferred_element_type=F32))

    def p3(b, carry):
        h2 = h_v[...]
        z1 = p3z(h2, 0)
        z1_v[rows(b, TB), :] = z1
        ln_zg(jnp.maximum(b - 1, 0), z1)
        p3wo(b + 1)
        zg = p3z(h2, FH)
        zg_v[0:TB, :] = zg
        ln_x1(b + 1, zg)
        return carry

    with _scope("p3"):
        lax.fori_loop(0, NB - 1, p3, 0)
        h2 = h_v[...]
        zl = zg_v[0:TB, :]
        zg = p3z(h2, FH)
        z2_v[rows(NB - 2, TB // 2), :] = _pack(_ln(zl))
        zg_v[0:TB, :] = zg
        z1 = p3z(h2, 0)
        z1_v[rows(NB - 1, TB), :] = z1
        ln_zg(NB - 1, z1)

    cp_wsp.wait()
    cp_wout.wait()

    NO = 4
    RO = TB4 // NO

    def ocopy(j):
        return pltpu.make_async_copy(out_v.at[rows(j, RO), :], out_hbm.at[rows(j, RO), :], osems.at[j])

    def p4(b, carry):
        g = jnp.dot(wsp_v[rows(b, TB4), :], _unpack(z2_v[...]), preferred_element_type=F32)
        g = g + jnp.concatenate([bcol_v[rows(b, TB4), :]] * (FH // 128), axis=1)
        u = (z1_v[rows(b, TB4), :] * g).astype(BF)
        for j in range(NO):
            y = jnp.dot(u[j * RO:(j + 1) * RO], wout_v[...], preferred_element_type=F32)
            r = rows(b * NO + j, RO)
            out_v[r, :] = (x1_v[r, :] + mod(5) * y).astype(BF)
            ocopy(b * NO + j).start()
        return carry

    with _scope("p4"):
        lax.fori_loop(0, S // TB4, p4, 0)
    with _scope("w_out"):
        for j in range(S // RO):
            ocopy(j).wait()


@jax.jit
def pallas_adaLN_cond__softmax_full_mha__mixer_gmlp__prompt_kernel(A_x, A_wqkv, A_wo, B_x, B_w_in, B_w_sp, B_b_sp, B_w_out, c, w_mod):
    x = A_x.reshape(S, D)
    bsp = B_b_sp.reshape(S // 128, 128)
    any_spec = pl.BlockSpec(memory_space=pl.ANY)
    out = pl.pallas_call(
        _kernel,
        out_shape=jax.ShapeDtypeStruct((S, D), BF),
        in_specs=[any_spec] * 9,
        out_specs=any_spec,
        scratch_shapes=[
            pltpu.VMEM((S, D), BF), pltpu.VMEM((D, 3 * D), BF), pltpu.VMEM((D, D), BF),
            pltpu.VMEM((D, 2 * FH), BF), pltpu.VMEM((S, S), BF), pltpu.VMEM((FH, D), BF),
            pltpu.VMEM((D, 6 * D), BF),
            pltpu.VMEM((8, 6 * D), F32),
            pltpu.VMEM((D, D), U32),
            pltpu.VMEM((TB // 2, D), U32),
            pltpu.VMEM((NP, S // 2, 128), U32),
            pltpu.VMEM((NB, D // 2, TB), U32),
            pltpu.VMEM((NC, D // 2, CK), U32),
            pltpu.VMEM((NI, S // 2, TQ), U32),
            pltpu.VMEM((NI, 8, TQ), F32),
            pltpu.VMEM((FEN + 9, 8, 128), F32),
            pltpu.VMEM((FEN + 9, 8, 128), F32),
            pltpu.VMEM((NI, DH, 8, TQ), F32),
            pltpu.VMEM((NB + 2, D, TB), F32),
            pltpu.VMEM((S, 128), F32),
            pltpu.VMEM((S + 8, D), F32),
            pltpu.VMEM((S, FH), F32),
            pltpu.VMEM((TB + 8, FH), F32),
            pltpu.VMEM((S // 2, FH), U32),
            pltpu.VMEM((S, D), BF),
            pltpu.VMEM((1, D), BF), pltpu.VMEM((S // 128, 128), BF),
            pltpu.SMEM((1,), jnp.int32),
            pltpu.SemaphoreType.DMA((11,)),
            pltpu.SemaphoreType.DMA((NB,)),
            pltpu.SemaphoreType.DMA((16,)),
        ],
        compiler_params=pltpu.CompilerParams(vmem_limit_bytes=110 * 1024 * 1024),
    )(c, bsp, x, A_wqkv, A_wo, B_w_in, B_w_sp, B_w_out, w_mod)
    return out.reshape(1, S, D)
```

```python
import jax
import jax.numpy as jnp
from jax import lax
import jax.experimental.pallas as pl
import jax.experimental.pallas.tpu as pltpu

S = 2048
D = 512
H = 32
DH = 16
FH = 896
EPS = 1e-5
LOG2E = 1.4426950408889634
BF = jnp.bfloat16
F32 = jnp.float32
U32 = jnp.uint32

TB = 256
NB = S // TB
U1 = 3
TB4 = 512
NO = 4
RO = TB4 // NO
RG = 16
TQ = 512
CK = 128
NQ = S // TQ
NC = S // CK
NP = H // 2
NI = 2 * NQ
FEN = 2 * NC * DH
QS, QE = 2, 11
S_LIMIT = 90.0
V_LIMIT = 2.0 ** 20
KP = 384
WO_STEPS = (0, 2, 4, 6, 8, 10, 12, 13, 14)
WO_STEPS0 = (4, 6, 8, 10, 11, 12, 13, 14, 15)
WO_ROWS = (0, 96, 192, 256)


def _ln(x):
    m = jnp.mean(x, axis=-1, keepdims=True)
    xc = x - m
    v = jnp.mean(xc * xc, axis=-1, keepdims=True)
    return xc * lax.rsqrt(v + EPS)


def _gelu(x):
    hx = 0.5 * x
    return hx + hx * jnp.tanh(x * (0.7978845608028654 + (0.7978845608028654 * 0.044715) * (x * x)))


def _pack(x):
    return pltpu.bitcast(x.astype(BF), U32)


def _unpack(x):
    return pltpu.bitcast(x, BF)


def _pk(a, b):
    return pltpu.pack_elementwise([a, b], packed_dtype=BF)


def _upk(x, i):
    return pltpu.unpack_elementwise(x, index=i, packed_dtype=BF, unpacked_dtype=F32)


def _mo(x, n):
    return x if isinstance(x, int) else pl.multiple_of(x, n)


def _rows(b, n):
    return pl.ds(_mo(b * n, n), n)


def _kernel(c_hbm, bsp_hbm, x_hbm, wqkv_hbm, wo_hbm, win_hbm, wsp_hbm, wout_hbm, wmod_hbm, out_hbm,
            x_v, wqkv_v, wo_v, win_v, wsp_v, wout_v, wmod_v,
            mod_v, wqvT_v, h_v, k_v, qT_v, vT_v, p_v, l_v, kba_v, kbb_v, qb_v, oT_v, scb_v, bs4_v,
            x1_v, z1_v, zg_v, zg2_v, z2_v, out_v, c_ref, bsp_ref, zero_s, sems, xsems, osems):
    def xcopy(b, sem):
        return pltpu.make_async_copy(x_hbm.at[_rows(b, TB), :], x_v.at[_rows(b, TB), :], sem)

    cp_mod_a = pltpu.make_async_copy(wmod_hbm.at[:, 0:2 * D], wmod_v.at[:, 0:2 * D], sems.at[0])
    cp_c = pltpu.make_async_copy(c_hbm, c_ref, sems.at[0])
    cp_x0 = xcopy(0, sems.at[1])
    cp_wq = pltpu.make_async_copy(wqkv_hbm.at[:, 0:D], wqkv_v.at[:, 0:D], sems.at[1])
    cp_wk = pltpu.make_async_copy(wqkv_hbm.at[:, D:2 * D], wqkv_v.at[:, D:2 * D], sems.at[2])
    cp_x1 = xcopy(1, sems.at[2])
    cp_mod_b = pltpu.make_async_copy(wmod_hbm.at[:, 2 * D:6 * D], wmod_v.at[:, 2 * D:6 * D], sems.at[3])
    cp_bsp = pltpu.make_async_copy(bsp_hbm, bsp_ref, sems.at[3])
    cp_wo = pltpu.make_async_copy(wo_hbm, wo_v, sems.at[3])
    cp_win = pltpu.make_async_copy(win_hbm, win_v, sems.at[4])
    cp_wsp = pltpu.make_async_copy(wsp_hbm, wsp_v, sems.at[4])
    cp_wout = pltpu.make_async_copy(wout_hbm, wout_v, sems.at[4])
    cp_wv = pltpu.make_async_copy(wqkv_hbm.at[:, 2 * D:3 * D], wqkv_v.at[:, 2 * D:3 * D], sems.at[5])

    cp_mod_a.start()
    cp_c.start()
    cp_x0.start()
    cp_wq.start()
    zero_s[0] = 0

    cp_c.wait()
    cp_mod_a.wait()
    cp_wk.start()
    c = c_ref[...].astype(F32)
    sc = (c * jax.nn.sigmoid(c)).astype(BF)
    scb_v[...] = jnp.broadcast_to(sc.astype(F32), (128, D)).T
    mod_v[:, 0:2 * D] = jnp.dot(jnp.broadcast_to(sc, (8, D)), wmod_v[:, 0:2 * D], preferred_element_type=F32)

    def mod(i):
        return mod_v[0:1, i * D:(i + 1) * D]

    qscale = (DH ** -0.5) * LOG2E

    def ln1(b):
        xw = pltpu.bitcast(x_v[_rows(b, TB), :], U32)
        he = _ln(_upk(xw, 0)) * (1.0 + mod(1)) + mod(0)
        ho = _ln(_upk(xw, 1)) * (1.0 + mod(1)) + mod(0)
        hn = _pk(he, ho)
        parts = []
        for g in range(TB // 16):
            if g % 8 == 7:
                parts.append(hn[g * 8:(g + 1) * 8])
            else:
                parts.append(_pack(jnp.concatenate([he[g * 8:(g + 1) * 8], ho[g * 8:(g + 1) * 8]], axis=0)))
        return hn, _unpack(jnp.concatenate(parts, axis=0))

    def kproj(b, hk, k2):
        k = jnp.dot(hk, wqkv_v[:, D:2 * D], preferred_element_type=F32)
        kp = _pack(k)
        for p in range(NP):
            blk = kp[:, (p // 4) * 128:(p // 4 + 1) * 128]
            if p % 4:
                blk = pltpu.roll(blk, 128 - 32 * (p % 4), 1)
            k_v[p, _rows(b, TB // 2), :] = blk
        return jnp.maximum(k2, jnp.max((k * k).reshape(TB // 8, 8, D), axis=0))

    def tproj(w, hn):
        return lax.dot_general(_unpack(w), _unpack(hn), (((1,), (1,)), ((), ())), preferred_element_type=F32)

    def qproj(b, hn, q2):
        q = tproj(wqvT_v[0:D // 2, :], hn) * qscale
        qp = _pack(q)
        for h in range(H):
            qT_v[h, b] = qp[h * 8:(h + 1) * 8]
        return jnp.maximum(q2, jnp.sum((q * q).reshape(H, DH, TB), axis=1))

    def vproj(b, hn, vm):
        v = tproj(wqvT_v[D // 2:D, :], hn)
        vp = _pack(v)
        for h in range(H):
            for j in range(TB // CK):
                vT_v[h, b * (TB // CK) + j] = vp[h * 8:(h + 1) * 8, j * CK:(j + 1) * CK]
        return jnp.maximum(vm, jnp.max(jnp.abs(v).reshape(D // 8, 8, TB), axis=0))

    zrows = jnp.zeros((8, TQ), U32)

    def qrows(pair, e, u):
        return jnp.concatenate([qT_v[pair * 2 + e, 2 * u], qT_v[pair * 2 + e, 2 * u + 1]], axis=1)

    def gen_kb(ref, pair, e, cg, b, ds):
        kf = _upk(k_v[pair, pl.ds(_mo(cg * 64 + 56, 8), 8), :], b)
        for d in ds:
            ref[(2 * cg + b) * DH + d] = jnp.broadcast_to(kf[:, e * DH + d:e * DH + d + 1], (8, 128))

    def gen_kb0(blk):
        for j in range(TB // CK):
            for b in range(2):
                gen_kb(kba_v, 0, 0, blk * (TB // CK) + j, b, range(DH))

    def gen_qb0(blk, es):
        for e in es:
            w = qT_v[e, blk]
            for i2 in range(2):
                wf = _upk(w, i2)
                for j in range(8):
                    qb_v[e, blk, 2 * j + i2] = jnp.broadcast_to(wf[j:j + 1, :], (8, TB))

    cp_x0.wait()
    cp_wq.wait()
    cp_x1.start()
    cp_wv.start()
    hn0, hk0 = ln1(0)
    wqvT_v[0:D // 2, :] = _pack(wqkv_v[:, 0:D].astype(F32).T)
    q2 = qproj(0, hn0, jnp.zeros((H, TB), F32))

    cp_wk.wait()
    cp_x1.wait()
    for b in range(2, 2 + U1):
        xcopy(b, xsems.at[b - 2]).start()
    k2 = kproj(0, hk0, jnp.zeros((8, D), F32))
    hn1, hk1 = ln1(1)
    h_v[...] = hn1

    cp_wv.wait()
    for b in range(2 + U1, NB):
        xcopy(b, xsems.at[b - 2]).start()
    cp_mod_b.start()
    cp_bsp.start()
    cp_wo.start()
    k2 = kproj(1, hk1, k2)
    wqvT_v[D // 2:D, :] = _pack(wqkv_v[:, 2 * D:3 * D].astype(F32).T)
    vm = vproj(0, hn0, jnp.zeros((8, TB), F32))
    gen_kb0(0)

    def p1(i, carry):
        k2, q2, vm = carry
        for t in range(U1):
            xcopy(i * U1 + t + 2, xsems.at[i * U1 + t]).wait()
        hn = h_v[...]
        for t in range(U1):
            b = i * U1 + t + 1
            hn2, hk2 = ln1(b + 1)
            q2 = qproj(b, hn, q2)
            k2 = kproj(b + 1, hk2, k2)
            vm = vproj(b, hn, vm)
            gen_kb0(b)
            gen_qb0(b - 1, (0, 1))
            hn = hn2
        h_v[...] = hn
        return k2, q2, vm

    k2, q2, vm = lax.fori_loop(0, (NB - 2) // U1, p1, (k2, q2, vm))

    cp_mod_b.wait()
    cp_bsp.wait()
    cp_wo.wait()
    for cp in (cp_win, cp_wsp, cp_wout):
        cp.start()
    q2 = qproj(NB - 1, h_v[...], q2)
    vm = vproj(NB - 1, h_v[...], vm)
    for j in range(2 * D // 128, 6 * D // 128):
        prod = wmod_v[:, j * 128:(j + 1) * 128].astype(F32) * scb_v[...]
        mod_v[0:1, j * 128:(j + 1) * 128] = jnp.sum(prod, axis=0, keepdims=True)
    gen_kb0(NB - 1)
    gen_qb0(NB - 2, (0,))
    gen_qb0(NB - 1, (0,))
    bs = bsp_ref[...].astype(F32)
    for j in range(S // TB4):
        bs4_v[j, 0:TB4 // 128, :] = bs[j * (TB4 // 128):(j + 1) * (TB4 // 128), :]

    k2 = jnp.max(k2, axis=0, keepdims=True)
    k2 = jnp.concatenate([k2[:, j * 128:(j + 1) * 128] for j in range(4)] * 2, axis=0)
    for sh in (1, 2, 4, 8):
        k2 = k2 + pltpu.roll(k2, sh, 1)
    lane = lax.broadcasted_iota(jnp.int32, (8, 128), 1)
    k2max = jnp.max(jnp.where(lane % 16 == 15, k2, 0.0))
    bound2 = jnp.max(q2) * k2max * 1.05
    safe = jnp.logical_and(bound2 <= S_LIMIT * S_LIMIT, jnp.max(vm) <= V_LIMIT)

    zero = zero_s[0]

    def outs(z, j, f):
        t = j * f * (z.shape[1] // 128) * (TB // 8) // (10 * (TB // RG))
        nt, r = divmod(t, TB // 8)
        return z[r * 8:(r + 1) * 8, nt * 128:(nt + 1) * 128]

    def oblk(b, lo, hi):
        return jnp.concatenate([oT_v[h, b] for h in range(lo // DH, hi // DH)], axis=0).T.astype(BF)

    def p3wo(b):
        a = jnp.dot(oblk(b, KP, D), wo_v[KP:D, :], preferred_element_type=F32)
        x1_v[_rows(b, TB), :] = x1_v[_rows(b, TB), :] + mod(2) * a

    def ln_x1_group(b, j, fence):
        if fence is not None:
            x1_v[pl.ds(pl.multiple_of(S + zero * 8, 8), 8), 0:128] = fence
        x1 = x1_v[pl.ds(_mo(b * TB + j * RG, RG), RG), :]
        h_v[j * RG // 2:(j + 1) * RG // 2, :] = _pack(_ln(x1) * (1.0 + mod(4)) + mod(3))

    def ln_x1(b, pace):
        for j in range(TB // RG):
            ln_x1_group(b, j, None if pace is None else outs(pace, j, 6))

    def put_o(head, u, o):
        oT_v[head, 2 * u] = o[:, :TB]
        oT_v[head, 2 * u + 1] = o[:, TB:]

    def group(pp, dump, pq, pn):
        pend = []
        for pos in range(NI):
            it = pos if pq is not None else (pos % 2) * NQ + pos // 2
            e, u = divmod(it, NQ)
            if pq is None and pos == 3:
                p3wo(0)
            kb_ref, kg_ref = (kba_v, kbb_v) if e == 0 else (kbb_v, kba_v)
            if pq is not None:
                blk = qrows(pq, e, u)
                qw = _unpack(jnp.concatenate([zrows, blk] if e else [blk, zrows], axis=0))
                gpair, ge = (pq, 1) if e == 0 else (pn, 0)
                slot = (it - 1) % NI
                w = qrows(pq if it == 0 else pn, slot // NQ, slot % NQ)
                for i2 in range(2):
                    wf = _upk(w, i2)
                    for j in range(4):
                        kb_ref[FEN + 1 + 4 * i2 + j] = wf[:, j * 128:(j + 1) * 128]
                qdone = 0
            lold = l_v[it]
            l = lv = acc = None
            if pq is None:
                ob = oblk(pos, 0, KP)
                wacc = None
            for c in range(NC):
                wsteps = WO_STEPS if pos else WO_STEPS0
                if pq is None and c in wsteps:
                    rb, kt = divmod(wsteps.index(c), KP // 128)
                    r0, r1 = WO_ROWS[rb], WO_ROWS[rb + 1]
                    w_ = jnp.dot(ob[r0:r1, kt * 128:(kt + 1) * 128],
                                 wo_v[kt * 128:(kt + 1) * 128, :], preferred_element_type=F32)
                    wacc = w_ if kt == 0 else w_ + wacc
                    if pos in (4, 5) and wsteps.index(c) < 8:
                        ln_x1_group(0, (pos - 4) * 8 + wsteps.index(c), w_[0:8, 0:128])
                    if kt == KP // 128 - 1:
                        r = slice(pos * TB + r0, pos * TB + r1)
                        x1_v[r, :] = x_v[r, :].astype(F32) + mod(2) * wacc
                x = p_v[it, c * 64:(c + 1) * 64, :]
                if pq is not None:
                    kc = _unpack(k_v[pq, c * 64:c * 64 + 56, :])[:, :2 * DH]
                    s = jnp.dot(kc, qw, preferred_element_type=F32)
                d_ = jnp.dot(_unpack(vT_v[pp * 2 + e, c]), _unpack(x), preferred_element_type=F32)
                acc = d_ if acc is None else d_ + acc
                if pq is not None:
                    for g in range(7):
                        p = jnp.exp2(s[g * 16:(g + 1) * 16])
                        t = p[:8] + p[8:]
                        l = t if l is None else l + t
                        p_v[it, c * 64 + g * 8:c * 64 + (g + 1) * 8, :] = _pk(p[:8], p[8:])
                    a = [None, None]
                    for d in range(DH):
                        if d % 4 == 0:
                            kb_ref[FEN + zero] = s[(d // 2) * 16 + 8:(d // 2) * 16 + 16, 0:128]
                        qb = jnp.concatenate([qb_v[e, 2 * u, d], qb_v[e, 2 * u + 1, d]], axis=1)
                        for b in range(2):
                            kb = kb_ref[(2 * c + b) * DH + d]
                            t = jnp.concatenate([kb] * (TQ // 128), axis=1) * qb
                            a[b] = t if a[b] is None else a[b] + t
                    a0 = jnp.exp2(a[0])
                    a1 = jnp.exp2(a[1])
                    lv = (a0 + a1) if lv is None else lv + (a0 + a1)
                    p_v[it, c * 64 + 56:c * 64 + 64, :] = _pk(a0, a1)
                if pend and c == 1:
                    pend.pop()()
                if pq is not None:
                    cg, part = divmod(u * NC + c, 4)
                    b, dh = divmod(part, 2)
                    gen_kb(kg_ref, gpair, ge, cg, b, range(dh * 8, dh * 8 + 8))
                    want = 0 if c < QS else min(DH, -(-DH * (c - QS + 1) // (QE - QS)))
                    for d in range(qdone, want):
                        src = jnp.concatenate([kb_ref[FEN + 1 + 4 * (d % 2) + j] for j in range(4)], axis=1)
                        row = jnp.broadcast_to(src[d // 2:d // 2 + 1, :], (8, TQ))
                        qb_v[slot // NQ, 2 * (slot % NQ), d] = row[:, :TB]
                        qb_v[slot // NQ, 2 * (slot % NQ) + 1, d] = row[:, TB:]
                    qdone = want

            def fin(it=it, e=e, u=u, acc=acc, l=l, lv=lv, lold=lold):
                ls = jnp.sum(lold, axis=0, keepdims=True)
                r0 = pl.reciprocal(ls, approx=True)
                r0 = r0 * (2.0 - ls * r0)
                put_o(pp * 2 + e, u if dump is None else jnp.where(dump, NQ, u), acc * r0)
                if pq is not None:
                    l_v[it] = l + lv

            if pos < NI - 1:
                pend.append(fin)
            else:
                fin()

    @pl.when(safe)
    def _bounded():
        def att(i, carry):
            group(jnp.maximum(i - 1, 0), i == 0, i, jnp.minimum(i + 1, NP - 1))
            return carry

        lax.fori_loop(0, NP, att, 0)
        group(NP - 1, None, None, None)

    @pl.when(jnp.logical_not(safe))
    def _exact_max():
        rgrp = lax.broadcasted_iota(jnp.int32, (16, TQ), 0) // 8

        def body(j, carry):
            h = j // NQ
            u = j % NQ
            pair = h // 2
            blk = jnp.concatenate([qrows(pair, 0, u), qrows(pair, 1, u)], axis=0)
            qw = _unpack(jnp.where(rgrp == h % 2, blk, jnp.zeros_like(blk)))

            def qk(c, mn):
                kc = _unpack(k_v[pair, _rows(c, 64), :])[:, :2 * DH]
                s = jnp.dot(kc, qw, preferred_element_type=F32)
                p_v[c // 8, _rows(c % 8, CK), :] = pltpu.bitcast(s, U32)
                return jnp.maximum(mn, jnp.max(s.reshape(CK // 8, 8, TQ), axis=0))

            mn = lax.fori_loop(0, NC, qk, jnp.full((8, TQ), -jnp.inf, F32))
            m = jnp.max(mn, axis=0, keepdims=True)

            def pv(c, carry):
                l, acc = carry
                x = pltpu.bitcast(p_v[c // 8, _rows(c % 8, CK), :], F32)
                parts = []
                for g in range(8):
                    p = jnp.exp2(x[g * 16:(g + 1) * 16] - m)
                    l = l + (p[:8] + p[8:])
                    parts.append(_pk(p[:8], p[8:]) if g < 7 else _pack(p))
                pb = _unpack(jnp.concatenate(parts, axis=0))
                return l, acc + jnp.dot(_unpack(vT_v[h, c]), pb, preferred_element_type=F32)

            l, acc = lax.fori_loop(0, NC, pv, (jnp.zeros((8, TQ), F32), jnp.zeros((DH, TQ), F32)))
            put_o(h, u, acc / jnp.sum(l, axis=0, keepdims=True))
            return carry

        lax.fori_loop(0, H * NQ, body, 0)

        def wo_part(b, carry):
            a = jnp.dot(oblk(b, 0, KP), wo_v[0:KP, :], preferred_element_type=F32)
            x1_v[_rows(b, TB), :] = x_v[_rows(b, TB), :].astype(F32) + mod(2) * a
            return carry

        lax.fori_loop(0, NB, wo_part, 0)
        p3wo(0)
        ln_x1(0, None)

    cp_win.wait()
    cp_wsp.wait()
    cp_wout.wait()

    def ln_zg(b, pace, ref):
        for j in range(TB // RG):
            ref[pl.ds(pl.multiple_of(TB + zero * 8, 8), 8), 0:128] = outs(pace, j, 8)
            z2_v[pl.ds(_mo(b * (TB // 2) + j * (RG // 2), RG // 2), RG // 2), :] = (
                _pack(_ln(ref[j * RG:(j + 1) * RG, :])))

    def p3z(h2, lo):
        return _gelu(jnp.dot(_unpack(h2), win_v[:, lo:lo + FH], preferred_element_type=F32))

    def p3(b, carry):
        h2 = h_v[...]
        z1 = p3z(h2, 0)
        z1_v[_rows(b, TB), :] = z1
        ln_zg(jnp.maximum(b - 1, 0), z1, zg_v)
        p3wo(b + 1)
        zg = p3z(h2, FH)
        zg_v[0:TB, :] = zg
        ln_x1(b + 1, zg)
        return carry

    lax.fori_loop(0, NB - 1, p3, 0)
    h2 = h_v[...]
    zg = p3z(h2, FH)
    zg2_v[0:TB, :] = zg
    ln_zg(NB - 2, zg, zg_v)
    z1 = p3z(h2, 0)
    z1_v[_rows(NB - 1, TB), :] = z1
    ln_zg(NB - 1, z1, zg2_v)

    def ocopy(j):
        return pltpu.make_async_copy(out_v.at[_rows(j, RO), :], out_hbm.at[_rows(j, RO), :], osems.at[0])

    def p4(b, carry):
        g = jnp.dot(wsp_v[_rows(b, TB4), :], _unpack(z2_v[...]), preferred_element_type=F32)
        bs = bs4_v[b, 0:TB4 // 128, :]
        bcol = jnp.concatenate([jnp.broadcast_to(bs[j:j + 1, :], (128, 128)).T for j in range(TB4 // 128)], axis=0)
        g = g + jnp.concatenate([bcol] * (FH // 128), axis=1)
        u = (z1_v[_rows(b, TB4), :] * g).astype(BF)
        for j in range(NO):
            y = jnp.dot(u[j * RO:(j + 1) * RO], wout_v[...], preferred_element_type=F32)
            r = _rows(b * NO + j, RO)
            out_v[r, :] = (x1_v[r, :] + mod(5) * y).astype(BF)
            ocopy(b * NO + j).start()
        return carry

    lax.fori_loop(0, S // TB4, p4, 0)
    for j in range(S // RO):
        ocopy(j).wait()


@jax.jit
def pallas_adaLN_cond__softmax_full_mha__mixer_gmlp__prompt_kernel(A_x, A_wqkv, A_wo, B_x, B_w_in, B_w_sp, B_b_sp, B_w_out, c, w_mod):
    x = A_x.reshape(S, D)
    bsp = B_b_sp.reshape(S // 128, 128)
    any_spec = pl.BlockSpec(memory_space=pl.ANY)
    out = pl.pallas_call(
        _kernel,
        out_shape=jax.ShapeDtypeStruct((S, D), BF),
        in_specs=[any_spec] * 9,
        out_specs=any_spec,
        scratch_shapes=[
            pltpu.VMEM((S, D), BF), pltpu.VMEM((D, 3 * D), BF), pltpu.VMEM((D, D), BF),
            pltpu.VMEM((D, 2 * FH), BF), pltpu.VMEM((S, S), BF), pltpu.VMEM((FH, D), BF),
            pltpu.VMEM((D, 6 * D), BF),
            pltpu.VMEM((8, 6 * D), F32),
            pltpu.VMEM((D, D), U32),
            pltpu.VMEM((TB // 2, D), U32),
            pltpu.VMEM((NP, S // 2, 128), U32),
            pltpu.VMEM((H, NB, 8, TB), U32),
            pltpu.VMEM((H, NC, 8, CK), U32),
            pltpu.VMEM((NI, S // 2, TQ), U32),
            pltpu.VMEM((NI, 8, TQ), F32),
            pltpu.VMEM((FEN + 9, 8, 128), F32),
            pltpu.VMEM((FEN + 9, 8, 128), F32),
            pltpu.VMEM((2, NB, DH, 8, TB), F32),
            pltpu.VMEM((H, 16, DH, TB), F32),
            pltpu.VMEM((D, 128), F32),
            pltpu.VMEM((S // TB4, 8, 128), F32),
            pltpu.VMEM((S + 8, D), F32),
            pltpu.VMEM((S, FH), F32),
            pltpu.VMEM((TB + 8, FH), F32),
            pltpu.VMEM((TB + 8, FH), F32),
            pltpu.VMEM((S // 2, FH), U32),
            pltpu.VMEM((S, D), BF),
            pltpu.VMEM((1, D), BF), pltpu.VMEM((S // 128, 128), BF),
            pltpu.SMEM((1,), jnp.int32),
            pltpu.SemaphoreType.DMA((6,)),
            pltpu.SemaphoreType.DMA((NB - 2,)),
            pltpu.SemaphoreType.DMA((1,)),
        ],
        compiler_params=pltpu.CompilerParams(vmem_limit_bytes=110 * 1024 * 1024),
    )(c, bsp, x, A_wqkv, A_wo, B_w_in, B_w_sp, B_w_out, w_mod)
    return out.reshape(1, S, D)
```

```python
import jax
import jax.numpy as jnp
from jax import lax
import jax.experimental.pallas as pl
import jax.experimental.pallas.tpu as pltpu

S = 2048
D = 512
H = 32
DH = 16
FH = 896
EPS = 1e-5
LOG2E = 1.4426950408889634
BF = jnp.bfloat16
F32 = jnp.float32
U32 = jnp.uint32

TB = 256
NB = S // TB
U1 = 3
TB4 = 512
NO = 4
RO = TB4 // NO
RG = 16
TQ = 512
CK = 128
NQ = S // TQ
NC = S // CK
NP = H // 2
NI = 2 * NQ
FEN = 2 * NC * DH
QS, QE = 2, 11
S_LIMIT = 90.0
V_LIMIT = 2.0 ** 20
KP = 384
WO_STEPS = (0, 2, 4, 6, 8, 10, 12, 13, 14)
WO_STEPS0 = (4, 6, 8, 10, 11, 12, 13, 14, 15)
WO_ROWS = (0, 96, 192, 256)


def _ln(x):
    m = jnp.mean(x, axis=-1, keepdims=True)
    xc = x - m
    v = jnp.mean(xc * xc, axis=-1, keepdims=True)
    return xc * lax.rsqrt(v + EPS)


def _gelu(x):
    hx = 0.5 * x
    return hx + hx * jnp.tanh(x * (0.7978845608028654 + (0.7978845608028654 * 0.044715) * (x * x)))


def _pack(x):
    return pltpu.bitcast(x.astype(BF), U32)


def _unpack(x):
    return pltpu.bitcast(x, BF)


def _mo(x, n):
    return x if isinstance(x, int) else pl.multiple_of(x, n)


def _rows(b, n):
    return pl.ds(_mo(b * n, n), n)


def _kernel(c_hbm, bsp_hbm, x_hbm, wqkv_hbm, wo_hbm, win_hbm, wsp_hbm, wout_hbm, wmod_hbm, out_hbm,
            x_v, wqkv_v, wo_v, win_v, wsp_v, wout_v, wmod_v,
            mod_v, wqvT_v, h_v, k_v, kf_v, qT_v, vT_v, p_v, s_v, l_v, kba_v, kbb_v, qb_v, oT_v, scb_v, bs4_v,
            x1_v, z1_v, zg_v, zg2_v, z2_v, out_v, c_ref, bsp_ref, zero_s, sems, xsems, osems):
    def xcopy(b, sem):
        return pltpu.make_async_copy(x_hbm.at[_rows(b, TB), :], x_v.at[_rows(b, TB), :], sem)

    cp_mod_a = pltpu.make_async_copy(wmod_hbm.at[:, 0:2 * D], wmod_v.at[:, 0:2 * D], sems.at[0])
    cp_c = pltpu.make_async_copy(c_hbm, c_ref, sems.at[0])
    cp_x0 = xcopy(0, sems.at[1])
    cp_wq = pltpu.make_async_copy(wqkv_hbm.at[:, 0:D], wqkv_v.at[:, 0:D], sems.at[1])
    cp_wk = pltpu.make_async_copy(wqkv_hbm.at[:, D:2 * D], wqkv_v.at[:, D:2 * D], sems.at[2])
    cp_x1 = xcopy(1, sems.at[2])
    cp_mod_b = pltpu.make_async_copy(wmod_hbm.at[:, 2 * D:6 * D], wmod_v.at[:, 2 * D:6 * D], sems.at[3])
    cp_bsp = pltpu.make_async_copy(bsp_hbm, bsp_ref, sems.at[3])
    cp_wo = pltpu.make_async_copy(wo_hbm, wo_v, sems.at[3])
    cp_win = pltpu.make_async_copy(win_hbm, win_v, sems.at[4])
    cp_wsp = pltpu.make_async_copy(wsp_hbm, wsp_v, sems.at[4])
    cp_wout = pltpu.make_async_copy(wout_hbm, wout_v, sems.at[4])
    cp_wv = pltpu.make_async_copy(wqkv_hbm.at[:, 2 * D:3 * D], wqkv_v.at[:, 2 * D:3 * D], sems.at[5])

    cp_mod_a.start()
    cp_c.start()
    cp_x0.start()
    cp_wq.start()
    zero_s[0] = 0

    cp_c.wait()
    cp_mod_a.wait()
    cp_wk.start()
    c = c_ref[...].astype(F32)
    sc = (c * jax.nn.sigmoid(c)).astype(BF)
    scb_v[...] = jnp.broadcast_to(sc.astype(F32), (128, D)).T
    mod_v[:, 0:2 * D] = jnp.dot(jnp.broadcast_to(sc, (8, D)), wmod_v[:, 0:2 * D], preferred_element_type=F32)

    def mod(i):
        return mod_v[0:1, i * D:(i + 1) * D]

    qscale = (DH ** -0.5) * LOG2E

    def ln1(b):
        return _pack(_ln(x_v[_rows(b, TB), :].astype(F32)) * (1.0 + mod(1)) + mod(0))

    def kproj(b, hn, k2):
        k = jnp.dot(_unpack(hn), wqkv_v[:, D:2 * D], preferred_element_type=F32)
        kp = _pack(k)
        kf = jnp.concatenate([k[j * CK + 112:(j + 1) * CK] for j in range(TB // CK)], axis=0).astype(BF).astype(F32)
        for p in range(NP):
            blk = kp[:, (p // 4) * 128:(p // 4 + 1) * 128]
            if p % 4:
                blk = pltpu.roll(blk, 128 - 32 * (p % 4), 1)
            k_v[p, _rows(b, TB // 2), :] = blk
            blk = kf[:, (p // 4) * 128:(p // 4 + 1) * 128]
            if p % 4:
                blk = pltpu.roll(blk, 128 - 32 * (p % 4), 1)
            kf_v[p, _rows(b, 32), :] = blk
        return jnp.maximum(k2, jnp.max((k * k).reshape(TB // 8, 8, D), axis=0))

    def tproj(w, hn):
        return lax.dot_general(_unpack(w), _unpack(hn), (((1,), (1,)), ((), ())), preferred_element_type=F32)

    def qproj(b, hn, q2):
        q = tproj(wqvT_v[0:D // 2, :], hn) * qscale
        qp = _pack(q)
        for h in range(H):
            qT_v[h, b] = qp[h * 8:(h + 1) * 8]
        return jnp.maximum(q2, jnp.sum((q * q).reshape(H, DH, TB), axis=1))

    def vproj(b, hn, vm):
        v = tproj(wqvT_v[D // 2:D, :], hn)
        vp = _pack(v)
        for h in range(H):
            for j in range(TB // CK):
                vT_v[h, b * (TB // CK) + j] = vp[h * 8:(h + 1) * 8, j * CK:(j + 1) * CK]
        return jnp.maximum(vm, jnp.max(jnp.abs(v).reshape(D // 8, 8, TB), axis=0))

    zrows = jnp.zeros((8, TQ), U32)

    def qrows(pair, e, u):
        return jnp.concatenate([qT_v[pair * 2 + e, 2 * u], qT_v[pair * 2 + e, 2 * u + 1]], axis=1)

    def gen_kb(ref, pair, e, cg, b, ds):
        kf = kf_v[pair, _rows(2 * cg + b, 8), :]
        for d in ds:
            ref[(2 * cg + b) * DH + d] = jnp.broadcast_to(kf[:, e * DH + d:e * DH + d + 1], (8, 128))

    def gen_kb0(blk):
        for j in range(TB // CK):
            for b in range(2):
                gen_kb(kba_v, 0, 0, blk * (TB // CK) + j, b, range(DH))

    def gen_qb0(blk, es):
        for e in es:
            wf = _unpack(qT_v[e, blk]).astype(F32)
            for d in range(DH):
                qb_v[e, blk, d] = jnp.broadcast_to(wf[d:d + 1, :], (8, TB))

    cp_x0.wait()
    cp_wq.wait()
    cp_x1.start()
    cp_wv.start()
    hn0 = ln1(0)
    wqvT_v[0:D // 2, :] = _pack(wqkv_v[:, 0:D].astype(F32).T)
    q2 = qproj(0, hn0, jnp.zeros((H, TB), F32))

    cp_wk.wait()
    cp_x1.wait()
    for b in range(2, 2 + U1):
        xcopy(b, xsems.at[b - 2]).start()
    k2 = kproj(0, hn0, jnp.zeros((8, D), F32))
    hn1 = ln1(1)
    h_v[...] = hn1

    cp_wv.wait()
    for b in range(2 + U1, NB):
        xcopy(b, xsems.at[b - 2]).start()
    cp_mod_b.start()
    cp_bsp.start()
    cp_wo.start()
    k2 = kproj(1, hn1, k2)
    wqvT_v[D // 2:D, :] = _pack(wqkv_v[:, 2 * D:3 * D].astype(F32).T)
    vm = vproj(0, hn0, jnp.zeros((8, TB), F32))
    gen_kb0(0)

    def p1(i, carry):
        k2, q2, vm = carry
        for t in range(U1):
            xcopy(i * U1 + t + 2, xsems.at[i * U1 + t]).wait()
        hn = h_v[...]
        for t in range(U1):
            b = i * U1 + t + 1
            hn2 = ln1(b + 1)
            q2 = qproj(b, hn, q2)
            k2 = kproj(b + 1, hn2, k2)
            vm = vproj(b, hn, vm)
            gen_kb0(b)
            gen_qb0(b - 1, (0, 1))
            hn = hn2
        h_v[...] = hn
        return k2, q2, vm

    k2, q2, vm = lax.fori_loop(0, (NB - 2) // U1, p1, (k2, q2, vm))

    cp_mod_b.wait()
    cp_bsp.wait()
    cp_wo.wait()
    for cp in (cp_win, cp_wsp, cp_wout):
        cp.start()
    q2 = qproj(NB - 1, h_v[...], q2)
    vm = vproj(NB - 1, h_v[...], vm)
    for j in range(2 * D // 128, 6 * D // 128):
        prod = wmod_v[:, j * 128:(j + 1) * 128].astype(F32) * scb_v[...]
        mod_v[0:1, j * 128:(j + 1) * 128] = jnp.sum(prod, axis=0, keepdims=True)
    gen_kb0(NB - 1)
    gen_qb0(NB - 2, (0,))
    gen_qb0(NB - 1, (0,))
    bs = bsp_ref[...].astype(F32)
    for j in range(S // TB4):
        bs4_v[j, 0:TB4 // 128, :] = bs[j * (TB4 // 128):(j + 1) * (TB4 // 128), :]

    k2 = jnp.max(k2, axis=0, keepdims=True)
    k2 = jnp.concatenate([k2[:, j * 128:(j + 1) * 128] for j in range(4)] * 2, axis=0)
    for sh in (1, 2, 4, 8):
        k2 = k2 + pltpu.roll(k2, sh, 1)
    lane = lax.broadcasted_iota(jnp.int32, (8, 128), 1)
    k2max = jnp.max(jnp.where(lane % 16 == 15, k2, 0.0))
    bound2 = jnp.max(q2) * k2max * 1.05
    safe = jnp.logical_and(bound2 <= S_LIMIT * S_LIMIT, jnp.max(vm) <= V_LIMIT)

    zero = jnp.clip(zero_s[0], 0, 1)

    def outs(z, j, f):
        t = j * f * (z.shape[1] // 128) * (TB // 8) // (10 * (TB // RG))
        nt, r = divmod(t, TB // 8)
        return z[r * 8:(r + 1) * 8, nt * 128:(nt + 1) * 128]

    def oblk(b, lo, hi):
        return jnp.concatenate([oT_v[h, b] for h in range(lo // DH, hi // DH)], axis=0).T.astype(BF)

    def p3wo(b):
        a = jnp.dot(oblk(b, KP, D), wo_v[KP:D, :], preferred_element_type=F32)
        x1_v[_rows(b, TB), :] = x1_v[_rows(b, TB), :] + mod(2) * a

    def ln_x1_group(b, j, fence):
        if fence is not None:
            x1_v[pl.ds(pl.multiple_of(S + zero * 8, 8), 8), 0:128] = fence
        x1 = x1_v[pl.ds(_mo(b * TB + j * RG, RG), RG), :]
        h_v[_rows(j, RG // 2), :] = _pack(_ln(x1) * (1.0 + mod(4)) + mod(3))

    def ln_x1(b, pace):
        for j in range(TB // RG):
            ln_x1_group(b, j, outs(pace, j, 6))

    def put_o(head, u, o):
        oT_v[head, 2 * u] = o[:, :TB]
        oT_v[head, 2 * u + 1] = o[:, TB:]

    def group(pp, dump, pq, pn):
        pend = []
        for pos in range(NI):
            it = pos if pq is not None else (pos % 2) * NQ + pos // 2
            e, u = divmod(it, NQ)
            if pq is None and pos == 3:
                p3wo(0)
            kb_ref, kg_ref = (kba_v, kbb_v) if e == 0 else (kbb_v, kba_v)
            if pq is not None:
                blk = qrows(pq, e, u)
                qw = _unpack(jnp.concatenate([zrows, blk] if e else [blk, zrows], axis=0))
                gpair, ge = (pq, 1) if e == 0 else (pn, 0)
                slot = (it - 1) % NI
                wf = _unpack(qrows(pq if it == 0 else pn, slot // NQ, slot % NQ)).astype(F32)
                for i2 in range(2):
                    for j in range(4):
                        kb_ref[FEN + 2 + 4 * i2 + j] = wf[i2 * 8:(i2 + 1) * 8, j * 128:(j + 1) * 128]
                qdone = 0
            lold = l_v[it]
            l = lv = acc = None
            if pq is None:
                ob = oblk(pos, 0, KP)
                wacc = None
            for c in range(NC):
                wsteps = WO_STEPS if pos else WO_STEPS0
                if pq is None and c in wsteps:
                    rb, kt = divmod(wsteps.index(c), KP // 128)
                    r0, r1 = WO_ROWS[rb], WO_ROWS[rb + 1]
                    w_ = jnp.dot(ob[r0:r1, kt * 128:(kt + 1) * 128],
                                 wo_v[kt * 128:(kt + 1) * 128, :], preferred_element_type=F32)
                    wacc = w_ if kt == 0 else w_ + wacc
                    if pos in (4, 5) and wsteps.index(c) < 8:
                        ln_x1_group(0, (pos - 4) * 8 + wsteps.index(c), w_[0:8, 0:128])
                    if kt == KP // 128 - 1:
                        r = slice(pos * TB + r0, pos * TB + r1)
                        x1_v[r, :] = x_v[r, :].astype(F32) + mod(2) * wacc
                x = p_v[it, c * CK:(c + 1) * CK, :]
                if pq is not None:
                    kc = _unpack(k_v[pq, c * 64:c * 64 + 56, :])[:, :2 * DH]
                    s = jnp.dot(kc, qw, preferred_element_type=F32)
                d_ = jnp.dot(_unpack(vT_v[pp * 2 + e, c]), x, preferred_element_type=F32)
                acc = d_ if acc is None else d_ + acc
                if pq is not None:
                    for g in range(7):
                        p = jnp.exp2(s[g * 16:(g + 1) * 16])
                        t = p[:8] + p[8:]
                        l = t if l is None else l + t
                        p_v[it, c * CK + g * 16:c * CK + (g + 1) * 16, :] = p.astype(BF)
                    a = [None, None]
                    for d in range(DH):
                        if d % 2 == 0:
                            f0 = min(d // 2, 6) * 16
                            kb_ref[FEN + zero] = s[f0:f0 + 8, 0:128]
                        qb = jnp.concatenate([qb_v[e, 2 * u, d], qb_v[e, 2 * u + 1, d]], axis=1)
                        for b in range(2):
                            kb = kb_ref[(2 * c + b) * DH + d]
                            t = jnp.concatenate([kb] * (TQ // 128), axis=1) * qb
                            a[b] = t if a[b] is None else a[b] + t
                    a0 = jnp.exp2(a[0])
                    a1 = jnp.exp2(a[1])
                    lv = (a0 + a1) if lv is None else lv + (a0 + a1)
                    p_v[it, c * CK + 112:c * CK + 128, :] = jnp.concatenate([a0, a1], axis=0).astype(BF)
                if pend and c == 1:
                    pend.pop()()
                if pq is not None:
                    cg, part = divmod(u * NC + c, 4)
                    b, dh = divmod(part, 2)
                    gen_kb(kg_ref, gpair, ge, cg, b, range(dh * 8, dh * 8 + 8))
                    want = 0 if c < QS else min(DH, -(-DH * (c - QS + 1) // (QE - QS)))
                    for d in range(qdone, want):
                        src = jnp.concatenate([kb_ref[FEN + 2 + 4 * (d // 8) + j] for j in range(4)], axis=1)
                        row = jnp.broadcast_to(src[d % 8:d % 8 + 1, :], (8, TQ))
                        qb_v[slot // NQ, 2 * (slot % NQ), d] = row[:, :TB]
                        qb_v[slot // NQ, 2 * (slot % NQ) + 1, d] = row[:, TB:]
                    qdone = want

            def fin(it=it, e=e, u=u, acc=acc, l=l, lv=lv, lold=lold):
                ls = jnp.sum(lold, axis=0, keepdims=True)
                r0 = pl.reciprocal(ls, approx=True)
                r0 = r0 * (2.0 - ls * r0)
                put_o(pp * 2 + e, u if dump is None else jnp.where(dump, NQ, u), acc * r0)
                if pq is not None:
                    l_v[it] = l + lv

            if pos < NI - 1:
                pend.append(fin)
            else:
                fin()

    @pl.when(safe)
    def _bounded():
        def att(i, carry):
            group(jnp.maximum(i - 1, 0), i == 0, i, jnp.minimum(i + 1, NP - 1))
            return carry

        lax.fori_loop(0, NP, att, 0)
        group(NP - 1, None, None, None)

    @pl.when(jnp.logical_not(safe))
    def _exact_max():
        rgrp = lax.broadcasted_iota(jnp.int32, (16, TQ), 0) // 8

        def body(j, carry):
            h = j // NQ
            u = j % NQ
            pair = h // 2
            blk = jnp.concatenate([qrows(pair, 0, u), qrows(pair, 1, u)], axis=0)
            qw = _unpack(jnp.where(rgrp == h % 2, blk, jnp.zeros_like(blk)))

            def qk(c, mn):
                kc = _unpack(k_v[pair, _rows(c, 64), :])[:, :2 * DH]
                s = jnp.dot(kc, qw, preferred_element_type=F32)
                s_v[_rows(c, CK), :] = s
                return jnp.maximum(mn, jnp.max(s.reshape(CK // 8, 8, TQ), axis=0))

            mn = lax.fori_loop(0, NC, qk, jnp.full((8, TQ), -jnp.inf, F32))
            m = jnp.max(mn, axis=0, keepdims=True)

            def pv(c, carry):
                l, acc = carry
                p = jnp.exp2(s_v[_rows(c, CK), :] - m)
                l = l + jnp.sum(p.reshape(CK // 8, 8, TQ), axis=0)
                pb = p.astype(BF)
                return l, acc + jnp.dot(_unpack(vT_v[h, c]), pb, preferred_element_type=F32)

            l, acc = lax.fori_loop(0, NC, pv, (jnp.zeros((8, TQ), F32), jnp.zeros((DH, TQ), F32)))
            put_o(h, u, acc / jnp.sum(l, axis=0, keepdims=True))
            return carry

        lax.fori_loop(0, H * NQ, body, 0)

        def wo_part(j, carry):
            nk = KP // 128
            b = jnp.where(j < NB * nk, j // nk, 0)
            kt = jnp.where(j < NB * nk, j % nk, nk)
            o = jnp.concatenate([oT_v[kt * 8 + h, b] for h in range(8)], axis=0).T.astype(BF)
            a = jnp.dot(o, wo_v[_rows(kt, 128), :], preferred_element_type=F32)
            base = jnp.where(kt == 0, x_v[_rows(b, TB), :].astype(F32), x1_v[_rows(b, TB), :])
            x1_v[_rows(b, TB), :] = base + mod(2) * a
            return carry

        lax.fori_loop(0, NB * (KP // 128) + 1, wo_part, 0)

        def ln_part(j, carry):
            ln_x1_group(0, j, None)
            return carry

        lax.fori_loop(0, TB // RG, ln_part, 0)

    cp_win.wait()
    cp_wsp.wait()
    cp_wout.wait()

    def ln_zg(b, pace, ref):
        for j in range(TB // RG):
            ref[pl.ds(pl.multiple_of(TB + zero * 8, 8), 8), 0:128] = outs(pace, j, 8)
            z2_v[pl.ds(_mo(b * (TB // 2) + j * (RG // 2), RG // 2), RG // 2), :] = (
                _pack(_ln(ref[j * RG:(j + 1) * RG, :])))

    def p3z(h2, lo):
        return _gelu(jnp.dot(_unpack(h2), win_v[:, lo:lo + FH], preferred_element_type=F32))

    def p3(b, carry):
        h2 = h_v[...]
        z1 = p3z(h2, 0)
        z1_v[_rows(b, TB), :] = z1
        ln_zg(jnp.maximum(b - 1, 0), z1, zg_v)
        p3wo(b + 1)
        zg = p3z(h2, FH)
        zg_v[0:TB, :] = zg
        ln_x1(b + 1, zg)
        return carry

    lax.fori_loop(0, NB - 1, p3, 0)
    h2 = h_v[...]
    zg = p3z(h2, FH)
    zg2_v[0:TB, :] = zg
    ln_zg(NB - 2, zg, zg_v)
    z1 = p3z(h2, 0)
    z1_v[_rows(NB - 1, TB), :] = z1
    ln_zg(NB - 1, z1, zg2_v)

    def ocopy(j):
        return pltpu.make_async_copy(out_v.at[_rows(j, RO), :], out_hbm.at[_rows(j, RO), :], osems.at[0])

    def p4(b, carry):
        g = jnp.dot(wsp_v[_rows(b, TB4), :], _unpack(z2_v[...]), preferred_element_type=F32)
        bs = bs4_v[b, 0:TB4 // 128, :]
        bcol = jnp.concatenate([jnp.broadcast_to(bs[j:j + 1, :], (128, 128)).T for j in range(TB4 // 128)], axis=0)
        g = g + jnp.concatenate([bcol] * (FH // 128), axis=1)
        u = (z1_v[_rows(b, TB4), :] * g).astype(BF)
        for j in range(NO):
            y = jnp.dot(u[j * RO:(j + 1) * RO], wout_v[...], preferred_element_type=F32)
            r = _rows(b * NO + j, RO)
            out_v[r, :] = (x1_v[r, :] + mod(5) * y).astype(BF)
            ocopy(b * NO + j).start()
        return carry

    lax.fori_loop(0, S // TB4, p4, 0)
    for j in range(S // RO):
        ocopy(j).wait()


@jax.jit
def pallas_adaLN_cond__softmax_full_mha__mixer_gmlp__prompt_kernel(A_x, A_wqkv, A_wo, B_x, B_w_in, B_w_sp, B_b_sp, B_w_out, c, w_mod):
    x = A_x.reshape(S, D)
    bsp = B_b_sp.reshape(S // 128, 128)
    any_spec = pl.BlockSpec(memory_space=pl.ANY)
    out = pl.pallas_call(
        _kernel,
        out_shape=jax.ShapeDtypeStruct((S, D), BF),
        in_specs=[any_spec] * 9,
        out_specs=any_spec,
        scratch_shapes=[
            pltpu.VMEM((S, D), BF), pltpu.VMEM((D, 3 * D), BF), pltpu.VMEM((D, D), BF),
            pltpu.VMEM((D, 2 * FH), BF), pltpu.VMEM((S, S), BF), pltpu.VMEM((FH, D), BF),
            pltpu.VMEM((D, 6 * D), BF),
            pltpu.VMEM((8, 6 * D), F32),
            pltpu.VMEM((D, D), U32),
            pltpu.VMEM((TB // 2, D), U32),
            pltpu.VMEM((NP, S // 2, 128), U32),
            pltpu.VMEM((NP, NC * 16, 128), F32),
            pltpu.VMEM((H, NB, 8, TB), U32),
            pltpu.VMEM((H, NC, 8, CK), U32),
            pltpu.VMEM((NI, S, TQ), BF),
            pltpu.VMEM((S, TQ), F32),
            pltpu.VMEM((NI, 8, TQ), F32),
            pltpu.VMEM((FEN + 10, 8, 128), F32),
            pltpu.VMEM((FEN + 10, 8, 128), F32),
            pltpu.VMEM((2, NB, DH, 8, TB), F32),
            pltpu.VMEM((H, 16, DH, TB), F32),
            pltpu.VMEM((D, 128), F32),
            pltpu.VMEM((S // TB4, 8, 128), F32),
            pltpu.VMEM((S + 16, D), F32),
            pltpu.VMEM((S, FH), F32),
            pltpu.VMEM((TB + 16, FH), F32),
            pltpu.VMEM((TB + 16, FH), F32),
            pltpu.VMEM((S // 2, FH), U32),
            pltpu.VMEM((S, D), BF),
            pltpu.VMEM((1, D), BF), pltpu.VMEM((S // 128, 128), BF),
            pltpu.SMEM((1,), jnp.int32),
            pltpu.SemaphoreType.DMA((6,)),
            pltpu.SemaphoreType.DMA((NB - 2,)),
            pltpu.SemaphoreType.DMA((1,)),
        ],
        compiler_params=pltpu.CompilerParams(vmem_limit_bytes=110 * 1024 * 1024),
    )(c, bsp, x, A_wqkv, A_wo, B_w_in, B_w_sp, B_w_out, w_mod)
    return out.reshape(1, S, D)
```

```python
import jax
import jax.numpy as jnp
from jax import lax
import jax.experimental.pallas as pl
import jax.experimental.pallas.tpu as pltpu

S = 2048
D = 512
H = 32
DH = 16
FH = 896
EPS = 1e-5
LOG2E = 1.4426950408889634
BF = jnp.bfloat16
F32 = jnp.float32
U32 = jnp.uint32

TB = 256
NB = S // TB
U1 = 3
TB4 = 512
NO = 4
RO = TB4 // NO
RG = 16
TQ = 512
CK = 128
NQ = S // TQ
NC = S // CK
NP = H // 2
NI = 2 * NQ
FEN = 2 * NC * DH
QS, QE = 3, 11
S_LIMIT = 90.0
V_LIMIT = 2.0 ** 20
KP = 384
WO_STEPS = (0, 2, 4, 6, 8, 10, 12, 13, 14)
WO_STEPS0 = (4, 6, 8, 10, 11, 12, 13, 14, 15)
WO_ROWS = (0, 96, 192, 256)


def _ln(x):
    m = jnp.mean(x, axis=-1, keepdims=True)
    xc = x - m
    v = jnp.mean(xc * xc, axis=-1, keepdims=True)
    return xc * lax.rsqrt(v + EPS)


def _gelu(x):
    hx = 0.5 * x
    return hx + hx * jnp.tanh(x * (0.7978845608028654 + (0.7978845608028654 * 0.044715) * (x * x)))


def _pack(x):
    return pltpu.bitcast(x.astype(BF), U32)


def _unpack(x):
    return pltpu.bitcast(x, BF)


def _stack(vals):
    return jnp.concatenate([v[None] for v in vals], axis=0)


def _mo(x, n):
    return x if isinstance(x, int) else pl.multiple_of(x, n)


def _rows(b, n):
    return pl.ds(_mo(b * n, n), n)


def _kernel(c_hbm, bsp_hbm, x_hbm, wqkv_hbm, wo_hbm, win_hbm, wsp_hbm, wout_hbm, wmod_hbm, out_hbm,
            x_v, wqkv_v, wo_v, win_v, wsp_v, wout_v, wmod_v,
            mod_v, wqvT_v, h_v, k_v, kf_v, qT_v, vT_v, p_v, s_v, l_v, kba_v, kbb_v, qb_v, oT_v, scb_v, bs4_v,
            x1_v, z1_v, zg_v, zg2_v, z2_v, out_v, c_ref, bsp_ref, zero_s, sems, xsems, osems):
    def xcopy(b, sem):
        return pltpu.make_async_copy(x_hbm.at[_rows(b, TB), :], x_v.at[_rows(b, TB), :], sem)

    cp_mod_a = pltpu.make_async_copy(wmod_hbm.at[:, 0:2 * D], wmod_v.at[:, 0:2 * D], sems.at[0])
    cp_c = pltpu.make_async_copy(c_hbm, c_ref, sems.at[0])
    cp_x0 = xcopy(0, sems.at[1])
    cp_wq = pltpu.make_async_copy(wqkv_hbm.at[:, 0:D], wqkv_v.at[:, 0:D], sems.at[1])
    cp_wk = pltpu.make_async_copy(wqkv_hbm.at[:, D:2 * D], wqkv_v.at[:, D:2 * D], sems.at[2])
    cp_x1 = xcopy(1, sems.at[2])
    cp_mod_b = pltpu.make_async_copy(wmod_hbm.at[:, 2 * D:6 * D], wmod_v.at[:, 2 * D:6 * D], sems.at[3])
    cp_bsp = pltpu.make_async_copy(bsp_hbm, bsp_ref, sems.at[3])
    cp_wo = pltpu.make_async_copy(wo_hbm, wo_v, sems.at[3])
    cp_win = pltpu.make_async_copy(win_hbm, win_v, sems.at[4])
    cp_wsp = pltpu.make_async_copy(wsp_hbm, wsp_v, sems.at[4])
    cp_wout = pltpu.make_async_copy(wout_hbm, wout_v, sems.at[4])
    cp_wv = pltpu.make_async_copy(wqkv_hbm.at[:, 2 * D:3 * D], wqkv_v.at[:, 2 * D:3 * D], sems.at[5])

    cp_mod_a.start()
    cp_c.start()
    cp_x0.start()
    cp_wq.start()
    zero_s[0] = 0

    cp_c.wait()
    cp_mod_a.wait()
    cp_wk.start()
    c = c_ref[...].astype(F32)
    sc = (c * jax.nn.sigmoid(c)).astype(BF)
    scb_v[...] = jnp.broadcast_to(sc.astype(F32), (128, D)).T
    mod_v[:, 0:2 * D] = jnp.dot(jnp.broadcast_to(sc, (8, D)), wmod_v[:, 0:2 * D], preferred_element_type=F32)

    def mod(i):
        return mod_v[0:1, i * D:(i + 1) * D]

    qscale = (DH ** -0.5) * LOG2E

    def ln1(b):
        return _pack(_ln(x_v[_rows(b, TB), :].astype(F32)) * (1.0 + mod(1)) + mod(0))

    def kproj(b, hn, k2):
        k = jnp.dot(_unpack(hn), wqkv_v[:, D:2 * D], preferred_element_type=F32)
        kp = _pack(k)
        kf = jnp.concatenate([k[j * CK + 112:(j + 1) * CK] for j in range(TB // CK)], axis=0).astype(BF).astype(F32)
        for p in range(NP):
            blk = kp[:, (p // 4) * 128:(p // 4 + 1) * 128]
            if p % 4:
                blk = pltpu.roll(blk, 128 - 32 * (p % 4), 1)
            k_v[p, _rows(b, TB // 2), :] = blk
            blk = kf[:, (p // 4) * 128:(p // 4 + 1) * 128]
            if p % 4:
                blk = pltpu.roll(blk, 128 - 32 * (p % 4), 1)
            kf_v[p, _rows(b, 32), :] = blk
        return jnp.maximum(k2, jnp.max((k * k).reshape(TB // 8, 8, D), axis=0))

    def tproj(w, hn):
        return lax.dot_general(_unpack(w), _unpack(hn), (((1,), (1,)), ((), ())), preferred_element_type=F32)

    def qproj(b, hn, q2):
        q = tproj(wqvT_v[0:D // 2, :], hn) * qscale
        qp = _pack(q)
        qT_v[:, b] = qp.reshape(H, 8, TB)
        return jnp.maximum(q2, jnp.sum((q * q).reshape(H, DH, TB), axis=1))

    def vproj(b, hn, vm):
        v = tproj(wqvT_v[D // 2:D, :], hn)
        vp = _pack(v)
        for j in range(TB // CK):
            vT_v[:, b * (TB // CK) + j] = vp[:, j * CK:(j + 1) * CK].reshape(H, 8, CK)
        return jnp.maximum(vm, jnp.max(jnp.abs(v).reshape(D // 8, 8, TB), axis=0))

    zrows = jnp.zeros((8, TQ), U32)

    def qrows(pair, e, u):
        return jnp.concatenate([qT_v[pair * 2 + e, 2 * u], qT_v[pair * 2 + e, 2 * u + 1]], axis=1)

    def gen_kb(ref, pair, e, cg, d0, nd):
        kf = kf_v[pair, _rows(cg, 16), :]
        vals = [jnp.broadcast_to(kf[b * 8:(b + 1) * 8, e * DH + d:e * DH + d + 1], (8, 128))
                for d in range(d0, d0 + nd) for b in range(2)]
        ref[pl.ds((cg * DH + d0) * 2, 2 * nd)] = _stack(vals)

    def gen_kb0(blk):
        for j in range(TB // CK):
            gen_kb(kba_v, 0, 0, blk * (TB // CK) + j, 0, DH)

    def gen_qb0(blk, es):
        for e in es:
            wf = _unpack(qT_v[e, blk]).astype(F32)
            qb_v[e, blk] = _stack([jnp.broadcast_to(wf[d:d + 1, :], (8, TB)) for d in range(DH)])

    cp_x0.wait()
    cp_wq.wait()
    cp_x1.start()
    cp_wv.start()
    hn0 = ln1(0)
    wqvT_v[0:D // 2, :] = _pack(wqkv_v[:, 0:D].astype(F32).T)
    q2 = qproj(0, hn0, jnp.zeros((H, TB), F32))

    cp_wk.wait()
    cp_x1.wait()
    for b in range(2, 2 + U1):
        xcopy(b, xsems.at[b - 2]).start()
    k2 = kproj(0, hn0, jnp.zeros((8, D), F32))
    hn1 = ln1(1)
    h_v[...] = hn1

    cp_wv.wait()
    for b in range(2 + U1, NB):
        xcopy(b, xsems.at[b - 2]).start()
    cp_mod_b.start()
    cp_bsp.start()
    cp_wo.start()
    k2 = kproj(1, hn1, k2)
    wqvT_v[D // 2:D, :] = _pack(wqkv_v[:, 2 * D:3 * D].astype(F32).T)
    vm = vproj(0, hn0, jnp.zeros((8, TB), F32))
    gen_kb0(0)

    def p1(i, carry):
        k2, q2, vm = carry
        for t in range(U1):
            xcopy(i * U1 + t + 2, xsems.at[i * U1 + t]).wait()
        hn = h_v[...]
        for t in range(U1):
            b = i * U1 + t + 1
            hn2 = ln1(b + 1)
            q2 = qproj(b, hn, q2)
            k2 = kproj(b + 1, hn2, k2)
            vm = vproj(b, hn, vm)
            gen_kb0(b)
            gen_qb0(b - 1, (0, 1))
            hn = hn2
        h_v[...] = hn
        return k2, q2, vm

    k2, q2, vm = lax.fori_loop(0, (NB - 2) // U1, p1, (k2, q2, vm))

    cp_mod_b.wait()
    cp_bsp.wait()
    cp_wo.wait()
    for cp in (cp_win, cp_wsp, cp_wout):
        cp.start()
    q2 = qproj(NB - 1, h_v[...], q2)
    vm = vproj(NB - 1, h_v[...], vm)
    for j in range(2 * D // 128, 6 * D // 128):
        prod = wmod_v[:, j * 128:(j + 1) * 128].astype(F32) * scb_v[...]
        mod_v[0:1, j * 128:(j + 1) * 128] = jnp.sum(prod, axis=0, keepdims=True)
    gen_kb0(NB - 1)
    gen_qb0(NB - 2, (0,))
    gen_qb0(NB - 1, (0,))
    bs = bsp_ref[...].astype(F32)
    for j in range(S // TB4):
        bs4_v[j, 0:TB4 // 128, :] = bs[j * (TB4 // 128):(j + 1) * (TB4 // 128), :]

    k2 = jnp.max(k2, axis=0, keepdims=True)
    k2 = jnp.concatenate([k2[:, j * 128:(j + 1) * 128] for j in range(4)] * 2, axis=0)
    for sh in (1, 2, 4, 8):
        k2 = k2 + pltpu.roll(k2, sh, 1)
    lane = lax.broadcasted_iota(jnp.int32, (8, 128), 1)
    k2max = jnp.max(jnp.where(lane % 16 == 15, k2, 0.0))
    bound2 = jnp.max(q2) * k2max * 1.05
    safe = jnp.logical_and(bound2 <= S_LIMIT * S_LIMIT, jnp.max(vm) <= V_LIMIT)

    zero = jnp.clip(zero_s[0], 0, 1)

    def outs(z, j, f):
        t = j * f * (z.shape[1] // 128) * (TB // 8) // (10 * (TB // RG))
        nt, r = divmod(t, TB // 8)
        return z[r * 8:(r + 1) * 8, nt * 128:(nt + 1) * 128]

    def oblk(b, lo, hi):
        return oT_v[lo // DH:hi // DH, b].reshape(hi - lo, TB).T.astype(BF)

    def p3wo(b):
        a = jnp.dot(oblk(b, KP, D), wo_v[KP:D, :], preferred_element_type=F32)
        x1_v[_rows(b, TB), :] = x1_v[_rows(b, TB), :] + mod(2) * a

    def ln_x1_group(b, j, fence):
        if fence is not None:
            x1_v[pl.ds(pl.multiple_of(S + zero * 8, 8), 8), 0:128] = fence
        x1 = x1_v[pl.ds(_mo(b * TB + j * RG, RG), RG), :]
        h_v[_rows(j, RG // 2), :] = _pack(_ln(x1) * (1.0 + mod(4)) + mod(3))

    def ln_x1(b, pace):
        for j in range(TB // RG):
            ln_x1_group(b, j, outs(pace, j, 6))

    def put_o(head, u, o):
        oT_v[head, 2 * u] = o[:, :TB]
        oT_v[head, 2 * u + 1] = o[:, TB:]

    def group(pp, dump, pq, pn):
        pend = []
        for pos in range(NI):
            it = pos if pq is not None else (pos % 2) * NQ + pos // 2
            e, u = divmod(it, NQ)
            if pq is None and pos == 3:
                p3wo(0)
            kb_ref, kg_ref = (kba_v, kbb_v) if e == 0 else (kbb_v, kba_v)
            if pq is not None:
                blk = qrows(pq, e, u)
                qw = _unpack(jnp.concatenate([zrows, blk] if e else [blk, zrows], axis=0))
                gpair, ge = (pq, 1) if e == 0 else (pn, 0)
                slot = (it - 1) % NI
                wf = _unpack(qrows(pq if it == 0 else pn, slot // NQ, slot % NQ)).astype(F32)
                kb_ref[FEN + 2:FEN + 10] = _stack(
                    [wf[i2 * 8:(i2 + 1) * 8, j * 128:(j + 1) * 128] for i2 in range(2) for j in range(4)])
                qdone = 0
            lold = l_v[it]
            l = lv = acc = None
            if pq is None:
                ob = oblk(pos, 0, KP)
                wacc = None
            for c in range(NC):
                wsteps = WO_STEPS if pos else WO_STEPS0
                if pq is None and c in wsteps:
                    rb, kt = divmod(wsteps.index(c), KP // 128)
                    r0, r1 = WO_ROWS[rb], WO_ROWS[rb + 1]
                    w_ = jnp.dot(ob[r0:r1, kt * 128:(kt + 1) * 128],
                                 wo_v[kt * 128:(kt + 1) * 128, :], preferred_element_type=F32)
                    wacc = w_ if kt == 0 else w_ + wacc
                    if pos in (4, 5) and wsteps.index(c) < 8:
                        ln_x1_group(0, (pos - 4) * 8 + wsteps.index(c), w_[0:8, 0:128])
                    if kt == KP // 128 - 1:
                        r = slice(pos * TB + r0, pos * TB + r1)
                        x1_v[r, :] = x_v[r, :].astype(F32) + mod(2) * wacc
                x = p_v[it, c * CK:(c + 1) * CK, :]
                if pq is not None:
                    kc = _unpack(k_v[pq, c * 64:c * 64 + 56, :])[:, :2 * DH]
                    s = jnp.dot(kc, qw, preferred_element_type=F32)
                d_ = jnp.dot(_unpack(vT_v[pp * 2 + e, c]), x, preferred_element_type=F32)
                acc = d_ if acc is None else d_ + acc
                if pq is not None:
                    p = jnp.exp2(s)
                    for g in range(7):
                        t = p[g * 16:g * 16 + 8] + p[g * 16 + 8:g * 16 + 16]
                        l = t if l is None else l + t
                    p_v[it, c * CK:c * CK + 112, :] = p.astype(BF)
                    a = None
                    for d0 in range(0, DH, 2):
                        f0 = min(d0 // 2, 6) * 16
                        kb_ref[FEN + zero] = s[f0:f0 + 8, 128:256]
                        kbs = jnp.concatenate([kb_ref[(c * DH + d0) * 2:(c * DH + d0) * 2 + 4]] * (TQ // 128), axis=2)
                        qbs = jnp.concatenate([qb_v[e, 2 * u, d0:d0 + 2], qb_v[e, 2 * u + 1, d0:d0 + 2]], axis=2)
                        for dd in range(2):
                            t = kbs[2 * dd:2 * dd + 2] * qbs[dd:dd + 1]
                            a = t if a is None else a + t
                    a = jnp.exp2(a.reshape(16, TQ))
                    a0, a1 = a[:8], a[8:]
                    lv = (a0 + a1) if lv is None else lv + (a0 + a1)
                    p_v[it, c * CK + 112:c * CK + 128, :] = a.astype(BF)
                if pend and c == 1:
                    pend.pop()()
                if pq is not None:
                    cg, part = divmod(u * NC + c, 4)
                    gen_kb(kg_ref, gpair, ge, cg, part * 4, 4)
                    want = 0 if c < QS else min(DH, -(-DH * (c - QS + 1) // (QE - QS)))
                    if want > qdone:
                        assert qdone // 8 == (want - 1) // 8
                        i2 = qdone // 8
                        st = kb_ref[FEN + 2 + 4 * i2:FEN + 6 + 4 * i2]
                        src = jnp.concatenate([st[j] for j in range(4)], axis=1)
                        rws = _stack([jnp.broadcast_to(src[d % 8:d % 8 + 1, :], (8, TQ)) for d in range(qdone, want)])
                        qb_v[slot // NQ, 2 * (slot % NQ), qdone:want] = rws[:, :, :TB]
                        qb_v[slot // NQ, 2 * (slot % NQ) + 1, qdone:want] = rws[:, :, TB:]
                    qdone = want

            def fin(it=it, e=e, u=u, acc=acc, l=l, lv=lv, lold=lold):
                ls = jnp.sum(lold, axis=0, keepdims=True)
                r0 = pl.reciprocal(ls, approx=True)
                r0 = r0 * (2.0 - ls * r0)
                put_o(pp * 2 + e, u if dump is None else jnp.where(dump, NQ, u), acc * r0)
                if pq is not None:
                    l_v[it] = l + lv

            if pos < NI - 1:
                pend.append(fin)
            else:
                fin()

    @pl.when(safe)
    def _bounded():
        def att(i, carry):
            group(jnp.maximum(i - 1, 0), i == 0, i, jnp.minimum(i + 1, NP - 1))
            return carry

        lax.fori_loop(0, NP, att, 0)
        group(NP - 1, None, None, None)

    @pl.when(jnp.logical_not(safe))
    def _exact_max():
        rgrp = lax.broadcasted_iota(jnp.int32, (16, TQ), 0) // 8

        def body(j, carry):
            h = j // NQ
            u = j % NQ
            pair = h // 2
            blk = jnp.concatenate([qrows(pair, 0, u), qrows(pair, 1, u)], axis=0)
            qw = _unpack(jnp.where(rgrp == h % 2, blk, jnp.zeros_like(blk)))

            def qk(c, mn):
                kc = _unpack(k_v[pair, _rows(c, 64), :])[:, :2 * DH]
                s = jnp.dot(kc, qw, preferred_element_type=F32)
                s_v[_rows(c, CK), :] = s
                return jnp.maximum(mn, jnp.max(s.reshape(CK // 8, 8, TQ), axis=0))

            mn = lax.fori_loop(0, NC, qk, jnp.full((8, TQ), -jnp.inf, F32))
            m = jnp.max(mn, axis=0, keepdims=True)

            def pv(c, carry):
                l, acc = carry
                p = jnp.exp2(s_v[_rows(c, CK), :] - m)
                l = l + jnp.sum(p.reshape(CK // 8, 8, TQ), axis=0)
                pb = p.astype(BF)
                return l, acc + jnp.dot(_unpack(vT_v[h, c]), pb, preferred_element_type=F32)

            l, acc = lax.fori_loop(0, NC, pv, (jnp.zeros((8, TQ), F32), jnp.zeros((DH, TQ), F32)))
            put_o(h, u, acc / jnp.sum(l, axis=0, keepdims=True))
            return carry

        lax.fori_loop(0, H * NQ, body, 0)

        def wo_part(j, carry):
            nk = KP // 128
            b = jnp.where(j < NB * nk, j // nk, 0)
            kt = jnp.where(j < NB * nk, j % nk, nk)
            o = oT_v[pl.ds(kt * 8, 8), b].reshape(128, TB).T.astype(BF)
            a = jnp.dot(o, wo_v[_rows(kt, 128), :], preferred_element_type=F32)
            base = jnp.where(kt == 0, x_v[_rows(b, TB), :].astype(F32), x1_v[_rows(b, TB), :])
            x1_v[_rows(b, TB), :] = base + mod(2) * a
            return carry

        lax.fori_loop(0, NB * (KP // 128) + 1, wo_part, 0)

        def ln_part(j, carry):
            ln_x1_group(0, j, None)
            return carry

        lax.fori_loop(0, TB // RG, ln_part, 0)

    cp_win.wait()
    cp_wsp.wait()
    cp_wout.wait()

    def ln_zg(b, pace, ref):
        for j in range(TB // RG):
            ref[pl.ds(pl.multiple_of(TB + zero * 8, 8), 8), 0:128] = outs(pace, j, 8)
            z2_v[pl.ds(_mo(b * (TB // 2) + j * (RG // 2), RG // 2), RG // 2), :] = (
                _pack(_ln(ref[j * RG:(j + 1) * RG, :])))

    def p3z(h2, lo):
        return _gelu(jnp.dot(_unpack(h2), win_v[:, lo:lo + FH], preferred_element_type=F32))

    def p3(b, carry):
        h2 = h_v[...]
        z1 = p3z(h2, 0)
        z1_v[_rows(b, TB), :] = z1
        ln_zg(jnp.maximum(b - 1, 0), z1, zg_v)
        p3wo(b + 1)
        zg = p3z(h2, FH)
        zg_v[0:TB, :] = zg
        ln_x1(b + 1, zg)
        return carry

    lax.fori_loop(0, NB - 1, p3, 0)
    h2 = h_v[...]
    zg = p3z(h2, FH)
    zg2_v[0:TB, :] = zg
    ln_zg(NB - 2, zg, zg_v)
    z1 = p3z(h2, 0)
    z1_v[_rows(NB - 1, TB), :] = z1
    ln_zg(NB - 1, z1, zg2_v)

    def ocopy(j):
        return pltpu.make_async_copy(out_v.at[_rows(j, RO), :], out_hbm.at[_rows(j, RO), :], osems.at[0])

    def p4(b, carry):
        g = jnp.dot(wsp_v[_rows(b, TB4), :], _unpack(z2_v[...]), preferred_element_type=F32)
        bs = bs4_v[b, 0:TB4 // 128, :]
        bcol = jnp.concatenate([jnp.broadcast_to(bs[j:j + 1, :], (128, 128)).T for j in range(TB4 // 128)], axis=0)
        g = g + jnp.concatenate([bcol] * (FH // 128), axis=1)
        u = (z1_v[_rows(b, TB4), :] * g).astype(BF)
        for j in range(NO):
            y = jnp.dot(u[j * RO:(j + 1) * RO], wout_v[...], preferred_element_type=F32)
            r = _rows(b * NO + j, RO)
            out_v[r, :] = (x1_v[r, :] + mod(5) * y).astype(BF)
            ocopy(b * NO + j).start()
        return carry

    lax.fori_loop(0, S // TB4, p4, 0)
    for j in range(S // RO):
        ocopy(j).wait()


@jax.jit
def pallas_adaLN_cond__softmax_full_mha__mixer_gmlp__prompt_kernel(A_x, A_wqkv, A_wo, B_x, B_w_in, B_w_sp, B_b_sp, B_w_out, c, w_mod):
    x = A_x.reshape(S, D)
    bsp = B_b_sp.reshape(S // 128, 128)
    any_spec = pl.BlockSpec(memory_space=pl.ANY)
    out = pl.pallas_call(
        _kernel,
        out_shape=jax.ShapeDtypeStruct((S, D), BF),
        in_specs=[any_spec] * 9,
        out_specs=any_spec,
        scratch_shapes=[
            pltpu.VMEM((S, D), BF), pltpu.VMEM((D, 3 * D), BF), pltpu.VMEM((D, D), BF),
            pltpu.VMEM((D, 2 * FH), BF), pltpu.VMEM((S, S), BF), pltpu.VMEM((FH, D), BF),
            pltpu.VMEM((D, 6 * D), BF),
            pltpu.VMEM((8, 6 * D), F32),
            pltpu.VMEM((D, D), U32),
            pltpu.VMEM((TB // 2, D), U32),
            pltpu.VMEM((NP, S // 2, 128), U32),
            pltpu.VMEM((NP, NC * 16, 128), F32),
            pltpu.VMEM((H, NB, 8, TB), U32),
            pltpu.VMEM((H, NC, 8, CK), U32),
            pltpu.VMEM((NI, S, TQ), BF),
            pltpu.VMEM((S, TQ), F32),
            pltpu.VMEM((NI, 8, TQ), F32),
            pltpu.VMEM((FEN + 10, 8, 128), F32),
            pltpu.VMEM((FEN + 10, 8, 128), F32),
            pltpu.VMEM((2, NB, DH, 8, TB), F32),
            pltpu.VMEM((H, 16, DH, TB), F32),
            pltpu.VMEM((D, 128), F32),
            pltpu.VMEM((S // TB4, 8, 128), F32),
            pltpu.VMEM((S + 16, D), F32),
            pltpu.VMEM((S, FH), F32),
            pltpu.VMEM((TB + 16, FH), F32),
            pltpu.VMEM((TB + 16, FH), F32),
            pltpu.VMEM((S // 2, FH), U32),
            pltpu.VMEM((S, D), BF),
            pltpu.VMEM((1, D), BF), pltpu.VMEM((S // 128, 128), BF),
            pltpu.SMEM((1,), jnp.int32),
            pltpu.SemaphoreType.DMA((6,)),
            pltpu.SemaphoreType.DMA((NB - 2,)),
            pltpu.SemaphoreType.DMA((1,)),
        ],
        compiler_params=pltpu.CompilerParams(vmem_limit_bytes=110 * 1024 * 1024),
    )(c, bsp, x, A_wqkv, A_wo, B_w_in, B_w_sp, B_w_out, w_mod)
    return out.reshape(1, S, D)
```

```python
import jax
import jax.numpy as jnp
from jax import lax
import jax.experimental.pallas as pl
import jax.experimental.pallas.tpu as pltpu

S = 2048
D = 512
H = 32
DH = 16
FH = 896
EPS = 1e-5
LOG2E = 1.4426950408889634
BF = jnp.bfloat16
F32 = jnp.float32
U32 = jnp.uint32

TB = 256
NB = S // TB
U1 = 3
TB4 = 512
NO = 4
RO = TB4 // NO
RG = 16
TQ = 512
CK = 128
NQ = S // TQ
NC = S // CK
NP = H // 2
NI = 2 * NQ
FEN = 2 * NC * DH
QS, QE = 3, 11
S_LIMIT = 90.0
V_LIMIT = 2.0 ** 20
KP = 384
WO_STEPS = (0, 2, 4, 6, 8, 10, 12, 13, 14)
WO_STEPS0 = (4, 6, 8, 10, 11, 12, 13, 14, 15)
WO_ROWS = (0, 96, 192, 256)


def _ln(x):
    m = jnp.mean(x, axis=-1, keepdims=True)
    xc = x - m
    v = jnp.mean(xc * xc, axis=-1, keepdims=True)
    return xc * lax.rsqrt(v + EPS)


def _gelu(x):
    hx = 0.5 * x
    return hx + hx * jnp.tanh(x * (0.7978845608028654 + (0.7978845608028654 * 0.044715) * (x * x)))


def _pack(x):
    return pltpu.bitcast(x.astype(BF), U32)


def _unpack(x):
    return pltpu.bitcast(x, BF)


def _stack(vals):
    return jnp.concatenate([v[None] for v in vals], axis=0)


def _mo(x, n):
    return x if isinstance(x, int) else pl.multiple_of(x, n)


def _rows(b, n):
    return pl.ds(_mo(b * n, n), n)


def _kernel(c_hbm, bsp_hbm, x_hbm, wqkv_hbm, wo_hbm, win_hbm, wsp_hbm, wout_hbm, wmod_hbm, out_hbm,
            x_v, wqkv_v, wo_v, win_v, wsp_v, wout_v, wmod_v,
            mod_v, wqvT_v, h_v, k_v, kf_v, qT_v, vT_v, p_v, s_v, l_v, kba_v, kbb_v, qb_v, oT_v, scb_v, bs4_v,
            x1_v, z1_v, zg_v, zg2_v, z2_v, out_v, c_ref, bsp_ref, zero_s, sems, xsems, osems):
    def xcopy(b, sem):
        return pltpu.make_async_copy(x_hbm.at[_rows(b, TB), :], x_v.at[_rows(b, TB), :], sem)

    cp_mod_a = pltpu.make_async_copy(wmod_hbm.at[:, 0:2 * D], wmod_v.at[:, 0:2 * D], sems.at[0])
    cp_c = pltpu.make_async_copy(c_hbm, c_ref, sems.at[0])
    cp_x0 = xcopy(0, sems.at[1])
    cp_wq = pltpu.make_async_copy(wqkv_hbm.at[:, 0:D], wqkv_v.at[:, 0:D], sems.at[1])
    cp_wk = pltpu.make_async_copy(wqkv_hbm.at[:, D:2 * D], wqkv_v.at[:, D:2 * D], sems.at[2])
    cp_x1 = xcopy(1, sems.at[2])
    cp_mod_b = pltpu.make_async_copy(wmod_hbm.at[:, 2 * D:6 * D], wmod_v.at[:, 2 * D:6 * D], sems.at[3])
    cp_bsp = pltpu.make_async_copy(bsp_hbm, bsp_ref, sems.at[3])
    cp_wo = pltpu.make_async_copy(wo_hbm, wo_v, sems.at[3])
    cp_win = pltpu.make_async_copy(win_hbm, win_v, sems.at[4])
    cp_wsp = pltpu.make_async_copy(wsp_hbm, wsp_v, sems.at[4])
    cp_wout = pltpu.make_async_copy(wout_hbm, wout_v, sems.at[4])
    cp_wv = pltpu.make_async_copy(wqkv_hbm.at[:, 2 * D:3 * D], wqkv_v.at[:, 2 * D:3 * D], sems.at[5])

    cp_mod_a.start()
    cp_c.start()
    cp_x0.start()
    cp_wq.start()
    zero_s[0] = 0

    cp_c.wait()
    cp_mod_a.wait()
    cp_wk.start()
    c = c_ref[...].astype(F32)
    sc = (c * jax.nn.sigmoid(c)).astype(BF)
    scb_v[...] = jnp.broadcast_to(sc.astype(F32), (128, D)).T
    mod_v[:, 0:2 * D] = jnp.dot(jnp.broadcast_to(sc, (8, D)), wmod_v[:, 0:2 * D], preferred_element_type=F32)

    def mod(i):
        return mod_v[0:1, i * D:(i + 1) * D]

    qscale = (DH ** -0.5) * LOG2E

    def ln1(b):
        return _pack(_ln(x_v[_rows(b, TB), :].astype(F32)) * (1.0 + mod(1)) + mod(0))

    def kproj(b, hn):
        k = jnp.dot(_unpack(hn), wqkv_v[:, D:2 * D], preferred_element_type=F32)
        kp = _pack(k)
        kf = jnp.concatenate([k[j * CK + 112:(j + 1) * CK] for j in range(TB // CK)], axis=0).astype(BF).astype(F32)
        for p in range(NP):
            blk = kp[:, (p // 4) * 128:(p // 4 + 1) * 128]
            if p % 4:
                blk = pltpu.roll(blk, 128 - 32 * (p % 4), 1)
            k_v[p, _rows(b, TB // 2), :] = blk
            blk = kf[:, (p // 4) * 128:(p // 4 + 1) * 128]
            if p % 4:
                blk = pltpu.roll(blk, 128 - 32 * (p % 4), 1)
            kf_v[p, _rows(b, 32), :] = blk
        return jnp.max((k * k).reshape(TB // 8, 8, D), axis=0)

    def knorm(w):
        w = jnp.concatenate([w[:, j * 128:(j + 1) * 128] for j in range(D // 128)], axis=0)
        for sh in (1, 2, 4, 8):
            w = w + pltpu.roll(w, sh, 1)
        return w

    def tproj(w, hn):
        return lax.dot_general(_unpack(w), _unpack(hn), (((1,), (1,)), ((), ())), preferred_element_type=F32)

    def qproj(b, hn, q2):
        q = tproj(wqvT_v[0:D // 2, :], hn) * qscale
        qp = _pack(q)
        qT_v[:, b] = qp.reshape(H, 8, TB)
        return jnp.maximum(q2, jnp.sum((q * q).reshape(H, DH, TB), axis=1))

    def vproj(b, hn, vm):
        v = tproj(wqvT_v[D // 2:D, :], hn)
        vp = _pack(v)
        for j in range(TB // CK):
            vT_v[:, b * (TB // CK) + j] = vp[:, j * CK:(j + 1) * CK].reshape(H, 8, CK)
        return jnp.maximum(vm, jnp.max(jnp.abs(v).reshape(D // 8, 8, TB), axis=0))

    zrows = jnp.zeros((8, TQ), U32)

    def qrows(pair, e, u):
        return jnp.concatenate([qT_v[pair * 2 + e, 2 * u], qT_v[pair * 2 + e, 2 * u + 1]], axis=1)

    def gen_kb(ref, pair, e, cg, d0, nd):
        kf = kf_v[pair, _rows(cg, 16), :]
        vals = [jnp.broadcast_to(kf[b * 8:(b + 1) * 8, e * DH + d:e * DH + d + 1], (8, 128))
                for d in range(d0, d0 + nd) for b in range(2)]
        ref[pl.ds((cg * DH + d0) * 2, 2 * nd)] = _stack(vals)

    def gen_kb0(blk):
        for j in range(TB // CK):
            gen_kb(kba_v, 0, 0, blk * (TB // CK) + j, 0, DH)

    def gen_qb0(blk, es):
        for e in es:
            wf = _unpack(qT_v[e, blk]).astype(F32)
            qb_v[e, blk] = _stack([jnp.broadcast_to(wf[d:d + 1, :], (8, TB)) for d in range(DH)])

    cp_x0.wait()
    cp_wq.wait()
    cp_x1.start()
    cp_wv.start()
    hn0 = ln1(0)
    wqvT_v[0:D // 2, :] = _pack(wqkv_v[:, 0:D].astype(F32).T)
    q2 = qproj(0, hn0, jnp.zeros((H, TB), F32))

    cp_wk.wait()
    cp_x1.wait()
    for b in range(2, 2 + U1):
        xcopy(b, xsems.at[b - 2]).start()
    kw0 = kproj(0, hn0)
    hn1 = ln1(1)
    h_v[...] = hn1

    cp_wv.wait()
    for b in range(2 + U1, NB):
        xcopy(b, xsems.at[b - 2]).start()
    cp_mod_b.start()
    cp_bsp.start()
    cp_wo.start()
    k2 = jnp.maximum(knorm(kw0), knorm(kproj(1, hn1)))
    wqvT_v[D // 2:D, :] = _pack(wqkv_v[:, 2 * D:3 * D].astype(F32).T)
    vm = vproj(0, hn0, jnp.zeros((8, TB), F32))
    gen_kb0(0)

    def p1(i, carry):
        k2, q2, vm = carry
        for t in range(U1):
            xcopy(i * U1 + t + 2, xsems.at[i * U1 + t]).wait()
        hn = h_v[...]
        for t in range(U1):
            b = i * U1 + t + 1
            hn2 = ln1(b + 1)
            q2 = qproj(b, hn, q2)
            k2 = jnp.maximum(k2, knorm(kproj(b + 1, hn2)))
            vm = vproj(b, hn, vm)
            gen_kb0(b)
            gen_qb0(b - 1, (0, 1))
            hn = hn2
        h_v[...] = hn
        return k2, q2, vm

    k2, q2, vm = lax.fori_loop(0, (NB - 2) // U1, p1, (k2, q2, vm))

    cp_mod_b.wait()
    cp_bsp.wait()
    cp_wo.wait()
    for cp in (cp_win, cp_wsp, cp_wout):
        cp.start()
    q2 = qproj(NB - 1, h_v[...], q2)
    vm = vproj(NB - 1, h_v[...], vm)
    for j in range(2 * D // 128, 6 * D // 128):
        prod = wmod_v[:, j * 128:(j + 1) * 128].astype(F32) * scb_v[...]
        mod_v[0:1, j * 128:(j + 1) * 128] = jnp.sum(prod, axis=0, keepdims=True)
    gen_kb0(NB - 1)
    gen_qb0(NB - 2, (0,))
    gen_qb0(NB - 1, (0,))
    bs = bsp_ref[...].astype(F32)
    for j in range(S // TB4):
        bs4_v[j, 0:TB4 // 128, :] = bs[j * (TB4 // 128):(j + 1) * (TB4 // 128), :]

    lane = lax.broadcasted_iota(jnp.int32, (32, 128), 1)
    k2max = jnp.max(jnp.where(lane % 16 == 15, k2, 0.0))
    bound2 = jnp.max(q2) * k2max * 1.05
    safe = jnp.logical_and(bound2 <= S_LIMIT * S_LIMIT, jnp.max(vm) <= V_LIMIT)

    zero = jnp.clip(zero_s[0], 0, 1)

    def outs(z, j, f):
        t = j * f * (z.shape[1] // 128) * (TB // 8) // (10 * (TB // RG))
        nt, r = divmod(t, TB // 8)
        return z[r * 8:(r + 1) * 8, nt * 128:(nt + 1) * 128]

    def oblk(b, lo, hi):
        return oT_v[lo // DH:hi // DH, b].reshape(hi - lo, TB).T.astype(BF)

    def p3wo(b):
        a = jnp.dot(oblk(b, KP, D), wo_v[KP:D, :], preferred_element_type=F32)
        x1_v[_rows(b, TB), :] = x1_v[_rows(b, TB), :] + mod(2) * a

    def ln_x1_group(b, j, fence):
        if fence is not None:
            x1_v[pl.ds(pl.multiple_of(S + zero * 8, 8), 8), 0:128] = fence
        x1 = x1_v[pl.ds(_mo(b * TB + j * RG, RG), RG), :]
        h_v[_rows(j, RG // 2), :] = _pack(_ln(x1) * (1.0 + mod(4)) + mod(3))

    def ln_x1(b, pace):
        for j in range(TB // RG):
            ln_x1_group(b, j, outs(pace, j, 6))

    def put_o(head, u, o):
        oT_v[head, 2 * u] = o[:, :TB]
        oT_v[head, 2 * u + 1] = o[:, TB:]

    def group(pp, dump, pq, pn):
        pend = []
        for pos in range(NI):
            it = pos if pq is not None else (pos % 2) * NQ + pos // 2
            e, u = divmod(it, NQ)
            if pq is None and pos == 3:
                p3wo(0)
            kb_ref, kg_ref = (kba_v, kbb_v) if e == 0 else (kbb_v, kba_v)
            if pq is not None:
                blk = qrows(pq, e, u)
                qw = _unpack(jnp.concatenate([zrows, blk] if e else [blk, zrows], axis=0))
                gpair, ge = (pq, 1) if e == 0 else (pn, 0)
                slot = (it - 1) % NI
                wf = _unpack(qrows(pq if it == 0 else pn, slot // NQ, slot % NQ)).astype(F32)
                kb_ref[FEN + 2:FEN + 10] = _stack(
                    [wf[i2 * 8:(i2 + 1) * 8, j * 128:(j + 1) * 128] for i2 in range(2) for j in range(4)])
                qdone = 0
            lold = l_v[it]
            l = lv = acc = None
            if pq is None:
                ob = oblk(pos, 0, KP)
                wacc = None
            for c in range(NC):
                wsteps = WO_STEPS if pos else WO_STEPS0
                if pq is None and c in wsteps:
                    rb, kt = divmod(wsteps.index(c), KP // 128)
                    r0, r1 = WO_ROWS[rb], WO_ROWS[rb + 1]
                    w_ = jnp.dot(ob[r0:r1, kt * 128:(kt + 1) * 128],
                                 wo_v[kt * 128:(kt + 1) * 128, :], preferred_element_type=F32)
                    wacc = w_ if kt == 0 else w_ + wacc
                    if pos in (4, 5) and wsteps.index(c) < 8:
                        ln_x1_group(0, (pos - 4) * 8 + wsteps.index(c), w_[0:8, 0:128])
                    if kt == KP // 128 - 1:
                        r = slice(pos * TB + r0, pos * TB + r1)
                        x1_v[r, :] = x_v[r, :].astype(F32) + mod(2) * wacc
                x = p_v[it, c * CK:(c + 1) * CK, :]
                if pq is not None:
                    kc = _unpack(k_v[pq, c * 64:c * 64 + 56, :])[:, :2 * DH]
                    s = jnp.dot(kc, qw, preferred_element_type=F32)
                d_ = jnp.dot(_unpack(vT_v[pp * 2 + e, c]), x, preferred_element_type=F32)
                acc = d_ if acc is None else d_ + acc
                if pq is not None:
                    p = jnp.exp2(s)
                    for g in range(7):
                        t = p[g * 16:g * 16 + 8] + p[g * 16 + 8:g * 16 + 16]
                        l = t if l is None else l + t
                    p_v[it, c * CK:c * CK + 112, :] = p.astype(BF)
                    a = None
                    for d0 in range(0, DH, 2):
                        f0 = min(d0 // 2, 6) * 16
                        kb_ref[FEN + zero] = s[f0:f0 + 8, 128:256]
                        kbs = jnp.concatenate([kb_ref[(c * DH + d0) * 2:(c * DH + d0) * 2 + 4]] * (TQ // 128), axis=2)
                        qbs = jnp.concatenate([qb_v[e, 2 * u, d0:d0 + 2], qb_v[e, 2 * u + 1, d0:d0 + 2]], axis=2)
                        for dd in range(2):
                            t = kbs[2 * dd:2 * dd + 2] * qbs[dd:dd + 1]
                            a = t if a is None else a + t
                    a = jnp.exp2(a.reshape(16, TQ))
                    a0, a1 = a[:8], a[8:]
                    lv = (a0 + a1) if lv is None else lv + (a0 + a1)
                    p_v[it, c * CK + 112:c * CK + 128, :] = a.astype(BF)
                if pend and c == 1:
                    pend.pop()()
                if pq is not None:
                    cg, part = divmod(u * NC + c, 4)
                    gen_kb(kg_ref, gpair, ge, cg, part * 4, 4)
                    want = 0 if c < QS else min(DH, -(-DH * (c - QS + 1) // (QE - QS)))
                    if want > qdone:
                        assert qdone // 8 == (want - 1) // 8
                        i2 = qdone // 8
                        st = kb_ref[FEN + 2 + 4 * i2:FEN + 6 + 4 * i2]
                        src = jnp.concatenate([st[j] for j in range(4)], axis=1)
                        rws = _stack([jnp.broadcast_to(src[d % 8:d % 8 + 1, :], (8, TQ)) for d in range(qdone, want)])
                        qb_v[slot // NQ, 2 * (slot % NQ), qdone:want] = rws[:, :, :TB]
                        qb_v[slot // NQ, 2 * (slot % NQ) + 1, qdone:want] = rws[:, :, TB:]
                    qdone = want

            def fin(it=it, e=e, u=u, acc=acc, l=l, lv=lv, lold=lold):
                ls = jnp.sum(lold, axis=0, keepdims=True)
                r0 = pl.reciprocal(ls, approx=True)
                r0 = r0 * (2.0 - ls * r0)
                put_o(pp * 2 + e, u if dump is None else jnp.where(dump, NQ, u), acc * r0)
                if pq is not None:
                    l_v[it] = l + lv

            if pos < NI - 1:
                pend.append(fin)
            else:
                fin()

    @pl.when(safe)
    def _bounded():
        def att(i, carry):
            group(jnp.maximum(i - 1, 0), i == 0, i, jnp.minimum(i + 1, NP - 1))
            return carry

        lax.fori_loop(0, NP, att, 0)
        group(NP - 1, None, None, None)

    @pl.when(jnp.logical_not(safe))
    def _exact_max():
        rgrp = lax.broadcasted_iota(jnp.int32, (16, TQ), 0) // 8

        def body(j, carry):
            h = j // NQ
            u = j % NQ
            pair = h // 2
            blk = jnp.concatenate([qrows(pair, 0, u), qrows(pair, 1, u)], axis=0)
            qw = _unpack(jnp.where(rgrp == h % 2, blk, jnp.zeros_like(blk)))

            def qk(c, mn):
                kc = _unpack(k_v[pair, _rows(c, 64), :])[:, :2 * DH]
                s = jnp.dot(kc, qw, preferred_element_type=F32)
                s_v[_rows(c, CK), :] = s
                return jnp.maximum(mn, jnp.max(s.reshape(CK // 8, 8, TQ), axis=0))

            mn = lax.fori_loop(0, NC, qk, jnp.full((8, TQ), -jnp.inf, F32))
            m = jnp.max(mn, axis=0, keepdims=True)

            def pv(c, carry):
                l, acc = carry
                p = jnp.exp2(s_v[_rows(c, CK), :] - m)
                l = l + jnp.sum(p.reshape(CK // 8, 8, TQ), axis=0)
                pb = p.astype(BF)
                return l, acc + jnp.dot(_unpack(vT_v[h, c]), pb, preferred_element_type=F32)

            l, acc = lax.fori_loop(0, NC, pv, (jnp.zeros((8, TQ), F32), jnp.zeros((DH, TQ), F32)))
            put_o(h, u, acc / jnp.sum(l, axis=0, keepdims=True))
            return carry

        lax.fori_loop(0, H * NQ, body, 0)

        def wo_part(j, carry):
            nk = KP // 128
            b = jnp.where(j < NB * nk, j // nk, 0)
            kt = jnp.where(j < NB * nk, j % nk, nk)
            o = oT_v[pl.ds(kt * 8, 8), b].reshape(128, TB).T.astype(BF)
            a = jnp.dot(o, wo_v[_rows(kt, 128), :], preferred_element_type=F32)
            base = jnp.where(kt == 0, x_v[_rows(b, TB), :].astype(F32), x1_v[_rows(b, TB), :])
            x1_v[_rows(b, TB), :] = base + mod(2) * a
            return carry

        lax.fori_loop(0, NB * (KP // 128) + 1, wo_part, 0)

        def ln_part(j, carry):
            ln_x1_group(0, j, None)
            return carry

        lax.fori_loop(0, TB // RG, ln_part, 0)

    cp_win.wait()
    cp_wsp.wait()
    cp_wout.wait()

    def ln_zg(b, pace, ref):
        for j in range(TB // RG):
            ref[pl.ds(pl.multiple_of(TB + zero * 8, 8), 8), 0:128] = outs(pace, j, 8)
            z2_v[pl.ds(_mo(b * (TB // 2) + j * (RG // 2), RG // 2), RG // 2), :] = (
                _pack(_ln(ref[j * RG:(j + 1) * RG, :])))

    def p3z(h2, lo):
        return _gelu(jnp.dot(_unpack(h2), win_v[:, lo:lo + FH], preferred_element_type=F32))

    def p3(b, carry):
        h2 = h_v[...]
        z1 = p3z(h2, 0)
        z1_v[_rows(b, TB), :] = z1
        ln_zg(jnp.maximum(b - 1, 0), z1, zg_v)
        p3wo(b + 1)
        zg = p3z(h2, FH)
        zg_v[0:TB, :] = zg
        ln_x1(b + 1, zg)
        return carry

    lax.fori_loop(0, NB - 1, p3, 0)
    h2 = h_v[...]
    zg = p3z(h2, FH)
    zg2_v[0:TB, :] = zg
    ln_zg(NB - 2, zg, zg_v)
    z1 = p3z(h2, 0)
    z1_v[_rows(NB - 1, TB), :] = z1
    ln_zg(NB - 1, z1, zg2_v)

    def ocopy(j):
        return pltpu.make_async_copy(out_v.at[_rows(j, RO), :], out_hbm.at[_rows(j, RO), :], osems.at[0])

    def p4(b, carry):
        g = jnp.dot(wsp_v[_rows(b, TB4), :], _unpack(z2_v[...]), preferred_element_type=F32)
        bs = bs4_v[b, 0:TB4 // 128, :]
        bcol = jnp.concatenate([jnp.broadcast_to(bs[j:j + 1, :], (128, 128)).T for j in range(TB4 // 128)], axis=0)
        g = g + jnp.concatenate([bcol] * (FH // 128), axis=1)
        u = (z1_v[_rows(b, TB4), :] * g).astype(BF)
        for j in range(NO):
            y = jnp.dot(u[j * RO:(j + 1) * RO], wout_v[...], preferred_element_type=F32)
            r = _rows(b * NO + j, RO)
            out_v[r, :] = (x1_v[r, :] + mod(5) * y).astype(BF)
            ocopy(b * NO + j).start()
        return carry

    lax.fori_loop(0, S // TB4, p4, 0)
    for j in range(S // RO):
        ocopy(j).wait()


@jax.jit
def pallas_adaLN_cond__softmax_full_mha__mixer_gmlp__prompt_kernel(A_x, A_wqkv, A_wo, B_x, B_w_in, B_w_sp, B_b_sp, B_w_out, c, w_mod):
    x = A_x.reshape(S, D)
    bsp = B_b_sp.reshape(S // 128, 128)
    any_spec = pl.BlockSpec(memory_space=pl.ANY)
    out = pl.pallas_call(
        _kernel,
        out_shape=jax.ShapeDtypeStruct((S, D), BF),
        in_specs=[any_spec] * 9,
        out_specs=any_spec,
        scratch_shapes=[
            pltpu.VMEM((S, D), BF), pltpu.VMEM((D, 3 * D), BF), pltpu.VMEM((D, D), BF),
            pltpu.VMEM((D, 2 * FH), BF), pltpu.VMEM((S, S), BF), pltpu.VMEM((FH, D), BF),
            pltpu.VMEM((D, 6 * D), BF),
            pltpu.VMEM((8, 6 * D), F32),
            pltpu.VMEM((D, D), U32),
            pltpu.VMEM((TB // 2, D), U32),
            pltpu.VMEM((NP, S // 2, 128), U32),
            pltpu.VMEM((NP, NC * 16, 128), F32),
            pltpu.VMEM((H, NB, 8, TB), U32),
            pltpu.VMEM((H, NC, 8, CK), U32),
            pltpu.VMEM((NI, S, TQ), BF),
            pltpu.VMEM((S, TQ), F32),
            pltpu.VMEM((NI, 8, TQ), F32),
            pltpu.VMEM((FEN + 10, 8, 128), F32),
            pltpu.VMEM((FEN + 10, 8, 128), F32),
            pltpu.VMEM((2, NB, DH, 8, TB), F32),
            pltpu.VMEM((H, 16, DH, TB), F32),
            pltpu.VMEM((D, 128), F32),
            pltpu.VMEM((S // TB4, 8, 128), F32),
            pltpu.VMEM((S + 16, D), F32),
            pltpu.VMEM((S, FH), F32),
            pltpu.VMEM((TB + 16, FH), F32),
            pltpu.VMEM((TB + 16, FH), F32),
            pltpu.VMEM((S // 2, FH), U32),
            pltpu.VMEM((S, D), BF),
            pltpu.VMEM((1, D), BF), pltpu.VMEM((S // 128, 128), BF),
            pltpu.SMEM((1,), jnp.int32),
            pltpu.SemaphoreType.DMA((6,)),
            pltpu.SemaphoreType.DMA((NB - 2,)),
            pltpu.SemaphoreType.DMA((1,)),
        ],
        compiler_params=pltpu.CompilerParams(vmem_limit_bytes=110 * 1024 * 1024),
    )(c, bsp, x, A_wqkv, A_wo, B_w_in, B_w_sp, B_w_out, w_mod)
    return out.reshape(1, S, D)
```
